```python
import jax
import jax.numpy as jnp

def _softmax(x, axis=-1):
    return jax.nn.softmax(x, axis=axis)
def _gelu(x):
    return jax.nn.gelu(x, approximate=True)
def _silu(x):
    return jax.nn.silu(x)
def _sigmoid(x):
    return jax.nn.sigmoid(x)
def _layernorm(x, axis=-1, eps=1e-5):
    m = jnp.mean(x, axis=axis, keepdims=True)
    v = jnp.var(x, axis=axis, keepdims=True)
    return (x - m) / jnp.sqrt(v + eps)
def _scatter_add(tgt, idx, src, axis=0):
    return tgt.at[idx].add(src)
def _segment_sum(src, seg, n):
    return jax.ops.segment_sum(src, seg, n)
class _Rng:
    def __init__(self, key):
        self._k = key
    def _next(self):
        self._k, sub = jax.random.split(self._k)
        return sub
    def normal(self, shape):
        return jax.random.normal(self._next(), shape, dtype=jnp.bfloat16)
    def randint(self, lo, hi, shape):
        return jax.random.randint(self._next(), shape, lo, hi, dtype=jnp.int32)
    def uniform(self, shape, lo=0.0, hi=1.0):
        return jax.random.uniform(self._next(), shape, jnp.bfloat16, lo, hi)
    def permutation(self, n):
        return jax.random.permutation(self._next(), n)


kernel_name = 'gated_mix__sliding_local_dilated__moe_arch_mod__prompt'

def setup_inputs():
    _rng = _Rng(jax.random.key(int.from_bytes(__import__("os").urandom(4), "little")))
    _w = (lambda a: (lambda t: t.astype(jnp.bfloat16) if jnp.issubdtype(t.dtype, jnp.floating) else t)(jnp.asarray(a)))
    def _A_setup():
        B, S, D = 1, 2048, 640
        return {
            "x": _w((lambda *s: _rng.normal(s) * 0.05)(B, S, D)),
            "wqkv": _w((lambda *s: _rng.normal(s) * 0.05)(D, 3 * D)),
            "wo": _w((lambda *s: _rng.normal(s) * 0.05)(D, D)),
        }
    _A_in = _A_setup()

    def _B_setup():
        B, S, D, F, C = 1, 2048, 640, 1728, 2
        return {
            "x": _w((lambda *s: _rng.normal(s) * 0.05)(B, S, D)),
            "w_r": _w((lambda *s: _rng.normal(s) * 0.05)(D)),
            "w_gate": _w((lambda *s: _rng.normal(s) * 0.05)(D, F)),
            "w_up": _w((lambda *s: _rng.normal(s) * 0.05)(D, F)),
            "w_down": _w((lambda *s: _rng.normal(s) * 0.05)(F, D)),
        }
    _B_in = _B_setup()

    return {
        "A_x": _A_in["x"],
        "A_wqkv": _A_in["wqkv"],
        "A_wo": _A_in["wo"],
        "B_x": _B_in["x"],
        "B_w_r": _B_in["w_r"],
        "B_w_gate": _B_in["w_gate"],
        "B_w_up": _B_in["w_up"],
        "B_w_down": _B_in["w_down"],
        "gate_w": _w((lambda *s: _rng.normal(s) * 0.05)(640)),
    }

def reference(A_x, A_wqkv, A_wo, B_x, B_w_r, B_w_gate, B_w_up, B_w_down, gate_w):
    def _A_ref(x, wqkv, wo):
        B, S, D = x.shape
        H = 32; Dh = D // H
        W, dil = 8, 2
        qkv = (lambda x, *d: x.transpose(*d))((x @ wqkv).reshape(B, S, 3, H, Dh), 2, 0, 3, 1, 4)
        q, k, v = qkv[0], qkv[1], qkv[2]
        scale = Dh ** -0.5
        pos = jnp.arange(S)
        off = jnp.arange(W) * dil
        idx = pos[:, None] - off[None, :]
        mask = idx >= 0
        idx_c = jnp.where(mask, idx, 0).reshape(-1)
        kg = k[:, :, idx_c, :].reshape(B, H, S, W, Dh)
        vg = v[:, :, idx_c, :].reshape(B, H, S, W, Dh)
        logits = jnp.einsum("bhsd,bhswd->bhsw", q, kg) * scale
        logits = jnp.where(mask[None, None, :, :], logits, -1e9)
        attn = _softmax(logits, axis=-1)
        o = jnp.einsum("bhsw,bhswd->bhsd", attn, vg)
        return (lambda x, *d: x.transpose(*d))(o, 0, 2, 1, 3).reshape(B, S, D) @ wo

    def _B_ref(x, w_r, w_gate, w_up, w_down):
        B, S, D = x.shape
        C = 2
        r = x @ w_r
        idx = jnp.argsort(-r, axis=-1)[:, :C]
        idx_e = jnp.repeat(idx.reshape(B, C, 1), D, axis=2)
        x_sel = jnp.take_along_axis(x, idx_e, axis=1)
        g = _silu(x_sel @ w_gate)
        u = x_sel @ w_up
        y = (g * u) @ w_down
        r_sel = _sigmoid(jnp.take_along_axis(r, idx, axis=1))
        y = y * r_sel.reshape(B, C, 1)
        b_off = (jnp.arange(B) * S).reshape(B, 1)
        flat_idx = (idx + b_off).reshape(B * C)
        zero = (x * 0.0).reshape(B * S, D)
        upd = _scatter_add(zero, flat_idx, y.reshape(B * C, D), axis=0)
        return x + upd.reshape(B, S, D)

    x = A_x
    g = _sigmoid((x * gate_w).sum(-1, keepdims=True))
    a = _A_ref(x, A_wqkv, A_wo)
    b = _B_ref(x, B_w_r, B_w_gate, B_w_up, B_w_down)
    return g * a + (1 - g) * b
```

```python
import functools
import math

import jax
import jax.numpy as jnp
import numpy as np
from jax.experimental import pallas as pl
from jax.experimental.pallas import tpu as pltpu

H = 32
WIN = 8
DIL = 2
HALO = 16
LANES = 128
F32 = jnp.float32
BF16 = jnp.bfloat16


def _sigmoid(x):
    return 1.0 / (1.0 + jnp.exp(-x))


def _dot_nt(a, b):
    return jax.lax.dot_general(a, b, (((1,), (1,)), ((), ())), preferred_element_type=F32)


def _kernel(ax_hbm, wqkv_hbm, wo_hbm, wr_ref, wg_hbm, wu_hbm, wd_hbm,
            gw_ref, out_hbm,
            ax_v, wqkv_v, wp_v, wo_v, wop_v, g_s, wg_v, wu_v, wd_v,
            q_s, k_s, v_s, o_s, out_v, t_s, r_s,
            sem_ax, sem_w, sem_misc, sem_out, *, S, D, TM, TB):
    DH = D // H
    NS = D // LANES
    NA = S // TM
    NB = S // TB
    scale = DH ** -0.5

    def ax_copy(i):
        rows = pl.ds(i * TM, TM)
        return pltpu.make_async_copy(ax_hbm.at[rows], ax_v.at[rows], sem_ax.at[i])

    def w_copy(c):
        cols = pl.ds(c * D, D)
        return pltpu.make_async_copy(wqkv_hbm.at[:, cols], wqkv_v.at[c], sem_w.at[c])

    wo_copy = pltpu.make_async_copy(wo_hbm, wo_v, sem_misc.at[0])
    wg_copy = pltpu.make_async_copy(wg_hbm, wg_v, sem_misc.at[1])
    wu_copy = pltpu.make_async_copy(wu_hbm, wu_v, sem_misc.at[2])
    wd_copy = pltpu.make_async_copy(wd_hbm, wd_v, sem_misc.at[3])

    def out_copy(i):
        rows = pl.ds(pl.multiple_of(i * TB, TB), TB)
        return pltpu.make_async_copy(out_v.at[rows], out_hbm.at[rows], sem_out.at[i])

    w_copy(0).start()
    ax_copy(0).start()
    w_copy(1).start()
    w_copy(2).start()
    for i in range(1, NA):
        ax_copy(i).start()
    wo_copy.start()
    wg_copy.start()
    wu_copy.start()
    wd_copy.start()

    def permute_cols(c):
        for r0 in range(0, D, 2 * LANES):
            nr = min(2 * LANES, D - r0)
            w32 = pltpu.bitcast(wqkv_v[c, r0:r0 + nr, :], jnp.int32)
            if nr < 2 * LANES:
                w32 = jnp.concatenate(
                    [w32, jnp.zeros((LANES - nr // 2, D), jnp.int32)], axis=0)
            t_s[...] = w32.T
            for s in range(NS):
                parts = [t_s[pl.ds(s * 4 + j, H, stride=DH), :] for j in range(4)]
                blk = jnp.concatenate(parts, axis=0).T
                wp_v[r0:r0 + nr, c * D + s * LANES:c * D + (s + 1) * LANES] = (
                    pltpu.bitcast(blk[:nr // 2], BF16))

    def permute_wo():
        for s in range(NS):
            cols = slice(s * LANES, (s + 1) * LANES)
            t_s[...] = pltpu.bitcast(wo_v[:, cols].astype(F32), jnp.int32)
            for d in range(DH):
                rows = pltpu.bitcast(t_s[pl.ds(d, H, stride=DH), :], F32)
                wop_v[d * H:(d + 1) * H, cols] = rows.astype(BF16)

    def qkv_part(i, c):
        row0 = pl.multiple_of(i * TM, TM)
        x = ax_v[pl.ds(row0, TM), :]
        res = jnp.dot(x, wp_v[:, c * D:(c + 1) * D], preferred_element_type=F32)
        dst, off = ((q_s, 0), (k_s, HALO), (v_s, HALO))[c]
        for s in range(NS):
            dst[s, pl.ds(row0 + off, TM), :] = res[:, s * LANES:(s + 1) * LANES]

    def attn_rows(row0, n, g0):
        q = [q_s[s, pl.ds(row0, n), :] for s in range(NS)]
        logits = []
        for w in range(WIN):
            base = row0 + (HALO - w * DIL)
            p = q[0] * k_s[0, pl.ds(base, n), :]
            for s in range(1, NS):
                p = p + q[s] * k_s[s, pl.ds(base, n), :]
            p = p + pltpu.roll(p, 64, 1)
            p = p + pltpu.roll(p, 32, 1)
            if g0 < w * DIL:
                pos = row0 + lax_iota((n, LANES), 0)
                p = jnp.where(pos >= w * DIL, p, -1e9 / scale)
            logits.append(p)
        m = logits[0]
        for w in range(1, WIN):
            m = jnp.maximum(m, logits[w])
        e = [jnp.exp2((l - m) * (scale * math.log2(math.e))) for l in logits]
        den = e[0]
        for w in range(1, WIN):
            den = den + e[w]
        inv = 1.0 / den
        for s in range(NS):
            acc = e[0] * v_s[s, pl.ds(row0 + HALO, n), :]
            for w in range(1, WIN):
                acc = acc + e[w] * v_s[s, pl.ds(row0 + (HALO - w * DIL), n), :]
            o_s[pl.ds(row0, n), s * LANES:(s + 1) * LANES] = (acc * inv).astype(BF16)

    def attn_block(i, lo, hi):
        row0 = pl.multiple_of(i * TM, TM)
        for g in range(lo, hi, 16):
            attn_rows(pl.multiple_of(row0 + g, 16), 16, g)

    def lax_iota(shape, dim):
        return jax.lax.broadcasted_iota(jnp.int32, shape, dim)

    def row_dot(x, w):
        p = x[:, :LANES] * w[:, :LANES]
        for s in range(1, NS):
            p = p + x[:, s * LANES:(s + 1) * LANES] * w[:, s * LANES:(s + 1) * LANES]
        return jnp.sum(p, axis=1, keepdims=True)

    def route_block(i):
        wr = wr_ref[...].astype(F32).reshape(1, D)
        gw = gw_ref[...].astype(F32).reshape(1, D)
        lane = lax_iota((8, LANES), 1)
        acc = jnp.full((8, LANES), -jnp.inf, F32)
        for g in range(0, TM, 16):
            rows = pl.ds(pl.multiple_of(i * TM + g, 16), 16)
            x = ax_v[rows, :].astype(F32)
            g_s[rows, :] = jnp.broadcast_to(_sigmoid(row_dot(x, gw)), (16, LANES))
            r = row_dot(x, wr)
            acc = jnp.where(lane == g // 8, r[:8], acc)
            acc = jnp.where(lane == g // 8 + 1, r[8:], acc)
        r_s[pl.ds(pl.multiple_of(i * 8, 8), 8), :] = acc

    for c in range(3):
        w_copy(c).wait()
        permute_cols(c)
        if c == 0:
            ax_copy(0).wait()
        qkv_part(0, c)
    route_block(0)
    for s in range(NS):
        k_s[s, 0:HALO, :] = jnp.broadcast_to(k_s[s, HALO:HALO + 1, :], (HALO, LANES))
        v_s[s, 0:HALO, :] = jnp.broadcast_to(v_s[s, HALO:HALO + 1, :], (HALO, LANES))

    cuts = [0, (TM // 48) * 16, (2 * TM // 48) * 16, TM]

    def body_a(i, carry):
        ax_copy(i).wait()
        for c in range(3):
            qkv_part(i, c)
            attn_block(i - 1, cuts[c], cuts[c + 1])
        route_block(i)
        return carry

    jax.lax.fori_loop(1, NA, body_a, 0)
    attn_block(NA - 1, 0, TM)

    wo_copy.wait()
    permute_wo()

    nr = NA * 8
    r = r_s[...].astype(BF16).astype(F32)
    r = jnp.where(r != r, -jnp.inf, r)
    sub = lax_iota((nr, LANES), 0)
    col = lax_iota((nr, LANES), 1)
    tok = jnp.where(col < TM // 8, (sub // 8) * TM + col * 8 + sub % 8, S - 1)
    m1 = jnp.max(r)
    i1 = jnp.min(jnp.where(r == m1, tok, S - 1))
    r2 = jnp.where(tok == i1, -jnp.inf, r)
    m2 = jnp.max(r2)
    i2 = jnp.min(jnp.where((r2 == m2) & (tok != i1), tok, S - 1))

    row16 = lax_iota((16, D), 0)

    def tile_of(i):
        return pl.ds(pl.multiple_of((i // 16) * 16, 16), 16)

    def pick(i):
        tile = ax_v[tile_of(i), :].astype(F32)
        return jnp.sum(jnp.where(row16 == i % 16, tile, 0.0), axis=0, keepdims=True)

    xsel = jnp.where(row16 == 0, pick(i1), jnp.where(row16 == 1, pick(i2), 0.0))
    xsel = xsel.astype(BF16)
    wg_copy.wait()
    wu_copy.wait()
    gg = _dot_nt(xsel, wg_v[...])
    uu = _dot_nt(xsel, wu_v[...])
    hh = (gg * _sigmoid(gg) * uu).astype(BF16)
    wd_copy.wait()
    y = jnp.dot(hh, wd_v[...], preferred_element_type=F32)
    for n, (i, m) in enumerate(((i1, m1), (i2, m2))):
        upd = y[n:n + 1, :] * _sigmoid(jnp.full((1, D), m, F32))
        tile = ax_v[tile_of(i), :].astype(F32)
        ax_v[tile_of(i), :] = jnp.where(row16 == i % 16, tile + upd, tile).astype(BF16)

    def body_c(i, carry):
        row0 = pl.multiple_of(i * TB, TB)
        a = jnp.dot(o_s[pl.ds(row0, TB), :], wop_v[...], preferred_element_type=F32)
        g = g_s[pl.ds(row0, TB), :]
        for s in range(NS):
            cols = slice(s * LANES, (s + 1) * LANES)
            b = ax_v[pl.ds(row0, TB), cols].astype(F32)
            out_v[pl.ds(row0, TB), cols] = (g * a[:, cols] + (1.0 - g) * b).astype(BF16)
        out_copy(i).start()
        return carry

    jax.lax.fori_loop(0, NB, body_c, 0)
    for i in range(NB):
        out_copy(i).wait()


@jax.jit
def pallas_gated_mix__sliding_local_dilated__moe_arch_mod__prompt_kernel(
    A_x: jax.Array,
    A_wqkv: jax.Array,
    A_wo: jax.Array,
    B_x: jax.Array,
    B_w_r: jax.Array,
    B_w_gate: jax.Array,
    B_w_up: jax.Array,
    B_w_down: jax.Array,
    gate_w: jax.Array,
):
    B, S, D = A_x.shape
    F = B_w_gate.shape[1]
    assert B == 1
    TM, TB = 256, 256
    NS = D // LANES
    hbm = pl.BlockSpec(memory_space=pltpu.HBM)
    vmem = pl.BlockSpec(memory_space=pltpu.VMEM)
    out = pl.pallas_call(
        functools.partial(_kernel, S=S, D=D, TM=TM, TB=TB),
        out_shape=jax.ShapeDtypeStruct((S, D), A_x.dtype),
        in_specs=[hbm, hbm, hbm, vmem, hbm, hbm, hbm, vmem],
        out_specs=hbm,
        scratch_shapes=[
            pltpu.VMEM((S, D), BF16),
            pltpu.VMEM((3, D, D), BF16),
            pltpu.VMEM((D, 3 * D), BF16),
            pltpu.VMEM((D, D), BF16),
            pltpu.VMEM((D, D), BF16),
            pltpu.VMEM((S, LANES), F32),
            pltpu.VMEM((F, D), BF16),
            pltpu.VMEM((F, D), BF16),
            pltpu.VMEM((F, D), BF16),
            pltpu.VMEM((NS, S, LANES), F32),
            pltpu.VMEM((NS, S + HALO, LANES), F32),
            pltpu.VMEM((NS, S + HALO, LANES), F32),
            pltpu.VMEM((S, D), BF16),
            pltpu.VMEM((S, D), BF16),
            pltpu.VMEM((D, LANES), jnp.int32),
            pltpu.VMEM((S // TM * 8, LANES), F32),
            pltpu.SemaphoreType.DMA((S // TM,)),
            pltpu.SemaphoreType.DMA((3,)),
            pltpu.SemaphoreType.DMA((4,)),
            pltpu.SemaphoreType.DMA((S // TB,)),
        ],
        compiler_params=pltpu.CompilerParams(vmem_limit_bytes=100 * 2**20),
    )(A_x.reshape(S, D), A_wqkv, A_wo, B_w_r,
      B_w_gate.T, B_w_up.T, B_w_down, gate_w)
    return out.reshape(B, S, D)
```

```python
import contextlib
import functools
import math

import jax
import jax.numpy as jnp
import numpy as np
from jax.experimental import pallas as pl
from jax.experimental.pallas import tpu as pltpu

H = 32
WIN = 8
DIL = 2
HALO = 16
LANES = 128
TM = 256
TO = 256
UNROLL_A = False
FLAGS = {}
NSPLIT = ((0, 15),)
SP = 32
LAG = 0
LEAD = 2
DYNW = 7
CH = 8
F32 = jnp.float32
BF16 = jnp.bfloat16


SCOPES = False


def _scope(name):
    return jax.named_scope(name) if SCOPES else contextlib.nullcontext()


def _sigmoid(x):
    return 1.0 / (1.0 + jnp.exp(-x))


def _dot_nt(a, b):
    return jax.lax.dot_general(a, b, (((1,), (1,)), ((), ())), preferred_element_type=F32)


def _iota(shape, dim):
    return jax.lax.broadcasted_iota(jnp.int32, shape, dim)


def _kernel(ax_hbm, wqkv_hbm, wo_hbm, wr_ref, wg_hbm, wu_hbm, wd_hbm,
            gw_ref, out_hbm,
            ax_v, wqkv_v, wp_v, wo_v, wop_v, wg_v, wu_v, wd_v,
            qkv_s, o_s, g_s, z_s, out_v, t_s, r_s,
            sem_ax, sem_w, sem_misc, sem_out, *, S, D):
    DH = D // H
    NS = D // LANES
    NA = S // TM
    qscale = DH ** -0.5 * math.log2(math.e)
    qkv_a, qkv_b = 0, 3 * NS
    GRP = LANES // H
    UNIT = 2 * LANES

    def ax_copy(i):
        rows = pl.ds(i * TM, TM)
        return pltpu.make_async_copy(ax_hbm.at[rows], ax_v.at[rows], sem_ax.at[i])

    def w_copy(c):
        cols = pl.ds(c * D, D)
        return pltpu.make_async_copy(wqkv_hbm.at[:, cols], wqkv_v.at[c], sem_w.at[c])

    def wq_copy(r0, r1):
        rows = pl.ds(r0, r1 - r0)
        return pltpu.make_async_copy(wqkv_hbm.at[rows, pl.ds(0, D)], wqkv_v.at[0, rows],
                                     sem_w.at[3 + r0 // UNIT])

    wo_copy = pltpu.make_async_copy(wo_hbm, wo_v, sem_misc.at[0])
    wg_copy = pltpu.make_async_copy(wg_hbm, wg_v, sem_misc.at[1])
    wu_copy = pltpu.make_async_copy(wu_hbm, wu_v, sem_misc.at[2])
    wd_copy = pltpu.make_async_copy(wd_hbm, wd_v, sem_misc.at[3])

    def out_copy(i):
        rows = pl.ds(i * TO, TO)
        return pltpu.make_async_copy(out_v.at[rows], out_hbm.at[rows], sem_out.at[i])

    def permute_unit(pieces):
        w32 = jnp.concatenate(
            [pltpu.bitcast(wqkv_v[c, r0:r0 + nr, :], jnp.int32) for c, r0, nr in pieces], axis=0)
        t_s[...] = w32.T
        for s in range(NS):
            parts = [t_s[pl.ds(s * GRP + j, H, stride=DH), :] for j in range(GRP)]
            blk = jnp.concatenate(parts, axis=0).T
            at = 0
            for c, r0, nr in pieces:
                wp_v[r0 // 2:(r0 + nr) // 2,
                     c * D + s * LANES:c * D + (s + 1) * LANES] = blk[at:at + nr // 2]
                at += nr // 2

    def permute_mxu(c, r0, nr):
        src = _iota((D, D), 0)
        dst = _iota((D, D), 1)
        perm = jnp.where(src == (dst % H) * DH + dst // H, 1.0, 0.0).astype(BF16)
        blk = jnp.dot(wqkv_v[c, r0:r0 + nr, :], perm, preferred_element_type=F32)
        wp_v[r0 // 2:(r0 + nr) // 2, c * D:(c + 1) * D] = pltpu.bitcast(
            blk.astype(BF16), jnp.int32)

    def permute_wo():
        for s in range(NS):
            cols = slice(s * LANES, (s + 1) * LANES)
            t_s[...] = pltpu.bitcast(wo_v[:, cols].astype(F32), jnp.int32)
            for d in range(DH):
                rows = pltpu.bitcast(t_s[pl.ds(d, H, stride=DH), :], F32)
                wop_v[d * H // 2:(d + 1) * H // 2, cols] = pltpu.bitcast(rows.astype(BF16), jnp.int32)

    def qkv_cols(i, lo, hi, buf):
        row0 = pl.multiple_of(i * TM, TM)
        x = ax_v[pl.ds(row0, TM), :]
        w = pltpu.bitcast(wp_v[:, lo * LANES:hi * LANES], BF16)
        res = jnp.dot(x, w, preferred_element_type=F32)
        for s in range(hi - lo):
            for r0 in range(0, TM, SP):
                piece = res[r0:r0 + SP, s * LANES:(s + 1) * LANES]
                if lo + s < NS:
                    piece = piece * qscale
                qkv_s[buf + lo + s, HALO + r0:HALO + r0 + SP, :] = piece
                yield

    def qkv_part(i, c, buf):
        for _ in qkv_cols(i, c * NS, (c + 1) * NS, buf):
            pass

    def copy_halo(src, dst):
        for s in range(NS, 3 * NS):
            qkv_s[dst + s, 0:HALO, :] = qkv_s[src + s, TM:TM + HALO, :]

    def attn_block(i, buf, z):
        row0 = pl.multiple_of(i * TM, TM)
        n = CH

        def shifted(slab, g, w):
            return qkv_s[buf + slab + (z if w >= DYNW else 0), pl.ds(HALO + g - w * DIL, n), :]

        def stage1(g):
            q = [qkv_s[buf + z + s, pl.ds(HALO + g, n), :] for s in range(NS)]
            out = []
            for w in range(WIN):
                p = q[0] * shifted(NS, g, w)
                for s in range(1, NS):
                    p = p + q[s] * shifted(NS + s, g, w)
                out.append((p, pltpu.roll(p, 2 * H, 1)))
            return out

        def stage2(g, st):
            out = []
            for p, pr in st:
                p = p + pr
                out.append((p, pltpu.roll(p, H, 1)))
            return out

        def stage3(g, st):
            logits = []
            for w, (p, pr) in enumerate(st):
                p = p + pr
                if g < w * DIL:
                    pos = row0 + g + _iota((n, LANES), 0)
                    p = jnp.where(pos >= w * DIL, p, -1e9 * math.log2(math.e))
                logits.append(p)
            m = logits[0]
            for w in range(1, WIN):
                m = jnp.maximum(m, logits[w])
            e = [jnp.exp2(l - m) for l in logits]
            den = e[0]
            for w in range(1, WIN):
                den = den + e[w]
            inv = 1.0 / den
            out = []
            for s in range(NS):
                acc = e[0] * shifted(2 * NS + s, g, 0)
                for w in range(1, WIN):
                    acc = acc + e[w] * shifted(2 * NS + s, g, w)
                out.append(acc * inv)
            return out

        groups = list(range(0, TM, n))
        s1, s2, pend = {}, {}, []
        for t in range(len(groups) + 2):
            if t < len(groups):
                s1[t] = stage1(groups[t])
            if 0 <= t - 1 < len(groups):
                s2[t - 1] = stage2(groups[t - 1], s1.pop(t - 1))
            if 0 <= t - 2 < len(groups):
                pend.append(stage3(groups[t - 2], s2.pop(t - 2)))
                if len(pend) * n >= 16:
                    g0 = groups[t - 2] + n - len(pend) * n
                    for s in range(NS):
                        o = jnp.concatenate([p[s] for p in pend], axis=0)
                        o_s[pl.ds(pl.multiple_of((row0 + g0) // 2, 8), len(pend) * n // 2),
                            s * LANES:(s + 1) * LANES] = pltpu.bitcast(o.astype(BF16), jnp.int32)
                    pend = []
            yield

    def row_dot(x, which):
        p = None
        for s in range(NS):
            w = qkv_s[6 * NS, pl.ds(pl.multiple_of((which + s) * 16, 16), 16), :]
            t = x[:, s * LANES:(s + 1) * LANES] * w
            p = t if p is None else p + t
        return jnp.sum(p, axis=1, keepdims=True)

    def route_block(i, z):
        lane = _iota((8, LANES), 1)
        acc = jnp.full((8, LANES), -jnp.inf, F32)
        for g in range(0, TM, 16):
            rows = pl.ds(pl.multiple_of(i * TM + g, 16), 16)
            x = ax_v[rows, :].astype(F32)
            r = row_dot(x, z)
            acc = jnp.where(lane == g // 8, r[:8], acc)
            acc = jnp.where(lane == g // 8 + 1, r[8:], acc)
            g_s[rows, :] = jnp.broadcast_to(_sigmoid(row_dot(x, z + NS)), (16, LANES))
            if g + 16 == TM:
                r_s[pl.ds(pl.multiple_of(i * 8, 8), 8), :] = acc
            yield

    wq_cuts = list(range(0, D, UNIT)) + [D]
    wq_parts = list(zip(wq_cuts[:-1], wq_cuts[1:]))
    for r0, r1 in wq_parts:
        wq_copy(r0, r1).start()
    ax_copy(0).start()
    w_copy(1).start()
    z_s[0] = 0
    for n, ref in enumerate((wr_ref, gw_ref)):
        w = ref[...].astype(F32).reshape(1, D)
        for s in range(NS):
            qkv_s[6 * NS, (n * NS + s) * 16:(n * NS + s + 1) * 16, :] = jnp.broadcast_to(
                w[:, s * LANES:(s + 1) * LANES], (16, LANES))
    tail0, tail = wq_parts[-1][0], D - wq_parts[-1][0]
    with _scope("perm0"):
        wq_copy(*wq_parts[0]).wait()
        w_copy(2).start()
        permute_unit([(0, 0, UNIT)])
        wq_copy(*wq_parts[1]).wait()
        wq_copy(*wq_parts[2]).wait()
        for i in range(1, NA):
            ax_copy(i).start()
        permute_unit([(0, UNIT, UNIT)])
        permute_mxu(0, tail0, tail)
    with _scope("wait_w1"):
        ax_copy(0).wait()
        w_copy(1).wait()
        w_copy(2).wait()
    wo_copy.start()
    wg_copy.start()
    wu_copy.start()
    wd_copy.start()
    with _scope("qkv0"):
        qkv_part(0, 0, qkv_a)
        permute_unit([(1, 0, UNIT)])
        permute_unit([(1, UNIT, UNIT)])
        permute_unit([(1, tail0, tail), (2, tail0, tail)])
        qkv_part(0, 1, qkv_a)
        permute_unit([(2, 0, UNIT)])
        permute_unit([(2, UNIT, UNIT)])
        qkv_part(0, 2, qkv_a)
        for _ in route_block(0, 0):
            pass
        for s in range(NS, 3 * NS):
            qkv_s[s, 0:HALO, :] = jnp.broadcast_to(qkv_s[s, HALO:HALO + 1, :], (HALO, LANES))

    def step_a(i, src, dst, route=True):
        copy_halo(src, dst)
        z = z_s[0]
        n_mm = 3 * NS * (TM // SP)
        jobs = [[attn_block(i - 1, src, z), TM // CH + 2, 0]]
        if route:
            jobs.append([route_block(i + 1, z), TM // 16, 0])
        k = 0
        for lo, hi in NSPLIT:
            for _ in qkv_cols(i, lo, hi, dst):
                k += 1
                for job in jobs:
                    upto = min(job[1], max(0, round((k - LAG) * job[1] / (n_mm - LAG - LEAD))))
                    for _ in range(upto - job[2]):
                        next(job[0])
                    job[2] = upto

    def body_a(j, carry):
        i = 2 * j + 1
        step_a(i, qkv_a, qkv_b)
        step_a(i + 1, qkv_b, qkv_a)
        return carry

    with _scope("wait_x"):
        for i in range(1, NA):
            ax_copy(i).wait()
    for _ in route_block(1, 0):
        pass
    with _scope("loopA"):
        if UNROLL_A:
            for j in range((NA - 2) // 2):
                body_a(j, 0)
        else:
            jax.lax.fori_loop(0, (NA - 2) // 2, body_a, 0)
    with _scope("wait_w"):
        wo_copy.wait()
        wg_copy.wait()
        wu_copy.wait()
        wd_copy.wait()

    nr = NA * 8
    r = r_s[...].astype(BF16).astype(F32)
    r = jnp.where(r != r, -jnp.inf, r)
    sub = _iota((nr, LANES), 0)
    col = _iota((nr, LANES), 1)
    tok = jnp.where(col < TM // 8, (sub // 8) * TM + col * 8 + sub % 8, S - 1)
    m1 = jnp.max(r)
    i1 = jnp.min(jnp.where(r == m1, tok, S - 1))
    r2 = jnp.where(tok == i1, -jnp.inf, r)
    m2 = jnp.max(r2)
    i2 = jnp.min(jnp.where((r2 == m2) & (tok != i1), tok, S - 1))

    row16 = _iota((16, D), 0)

    def tile_of(i):
        return pl.ds(pl.multiple_of((i // 16) * 16, 16), 16)

    def pick(i):
        tile = ax_v[tile_of(i), :].astype(F32)
        return jnp.sum(jnp.where(row16 == i % 16, tile, 0.0), axis=0, keepdims=True)

    xsel = jnp.where(row16 == 0, pick(i1), jnp.where(row16 == 1, pick(i2), 0.0))
    xsel = xsel.astype(BF16)
    gg = _dot_nt(xsel, wg_v[...])
    uu = _dot_nt(xsel, wu_v[...])
    hh = (gg * _sigmoid(gg) * uu).astype(BF16)
    y = jnp.dot(hh, wd_v[...], preferred_element_type=F32)
    permute_wo()
    step_a(NA - 1, qkv_a, qkv_b, route=False)
    for n, (i, m) in enumerate(((i1, m1), (i2, m2))):
        upd = y[n:n + 1, :] * _sigmoid(jnp.full((1, D), m, F32))
        tile = ax_v[tile_of(i), :].astype(F32)
        ax_v[tile_of(i), :] = jnp.where(row16 == i % 16, tile + upd, tile).astype(BF16)

    def out_block(i):
        row0 = i * TM
        o = pltpu.bitcast(o_s[row0 // 2:(row0 + TM) // 2, :], BF16)
        a = jnp.dot(o, pltpu.bitcast(wop_v[...], BF16), preferred_element_type=F32)
        g = g_s[row0:row0 + TM, :]
        for s in range(NS):
            cols = slice(s * LANES, (s + 1) * LANES)
            b = ax_v[row0:row0 + TM, cols].astype(F32)
            out_v[row0:row0 + TM, cols] = (g * a[:, cols] + (1.0 - g) * b).astype(BF16)
        for t in range(row0 // TO, (row0 + TM) // TO):
            out_copy(t).start()

    with _scope("phaseC"):
        for _ in attn_block(NA - 1, qkv_b, 0):
            pass
        for i in range(NA):
            out_block(i)
    with _scope("drain"):
        for t in range(S // TO):
            out_copy(t).wait()


@jax.jit
def pallas_gated_mix__sliding_local_dilated__moe_arch_mod__prompt_kernel(
    A_x: jax.Array,
    A_wqkv: jax.Array,
    A_wo: jax.Array,
    B_x: jax.Array,
    B_w_r: jax.Array,
    B_w_gate: jax.Array,
    B_w_up: jax.Array,
    B_w_down: jax.Array,
    gate_w: jax.Array,
):
    B, S, D = A_x.shape
    F = B_w_gate.shape[1]
    assert B == 1
    NS = D // LANES
    hbm = pl.BlockSpec(memory_space=pltpu.HBM)
    vmem = pl.BlockSpec(memory_space=pltpu.VMEM)
    out = pl.pallas_call(
        functools.partial(_kernel, S=S, D=D),
        out_shape=jax.ShapeDtypeStruct((S, D), A_x.dtype),
        in_specs=[hbm, hbm, hbm, vmem, hbm, hbm, hbm, vmem],
        out_specs=hbm,
        scratch_shapes=[
            pltpu.VMEM((S, D), BF16),
            pltpu.VMEM((3, D, D), BF16),
            pltpu.VMEM((D // 2, 3 * D), jnp.int32),
            pltpu.VMEM((D, D), BF16),
            pltpu.VMEM((D // 2, D), jnp.int32),
            pltpu.VMEM((F, D), BF16),
            pltpu.VMEM((F, D), BF16),
            pltpu.VMEM((F, D), BF16),
            pltpu.VMEM((6 * NS + 1, HALO + TM, LANES), F32),
            pltpu.VMEM((S // 2, D), jnp.int32),
            pltpu.VMEM((S, LANES), F32),
            pltpu.SMEM((1,), jnp.int32),
            pltpu.VMEM((S, D), BF16),
            pltpu.VMEM((D, LANES), jnp.int32),
            pltpu.VMEM((S // TM * 8, LANES), F32),
            pltpu.SemaphoreType.DMA((S // TM,)),
            pltpu.SemaphoreType.DMA((6,)),
            pltpu.SemaphoreType.DMA((4,)),
            pltpu.SemaphoreType.DMA((S // TO,)),
        ],
        compiler_params=pltpu.CompilerParams(vmem_limit_bytes=100 * 2**20, flags=FLAGS),
    )(A_x.reshape(S, D), A_wqkv, A_wo, B_w_r,
      B_w_gate.T, B_w_up.T, B_w_down, gate_w)
    return out.reshape(B, S, D)
```

```python
import contextlib
import functools
import math

import jax
import jax.numpy as jnp
import numpy as np
from jax.experimental import pallas as pl
from jax.experimental.pallas import tpu as pltpu

H = 32
WIN = 8
DIL = 2
HALO = 16
LANES = 128
TM = 256
OUT_CUTS = (0, 256, 512, 768, 1024, 1280, 1536, 1792, 1920, 1984, 2048)
FENCE = 0
FLAGS = {}
SP = 16
LAG = 0
LEAD = 4
DYNW = 7
CH = 8
F32 = jnp.float32
BF16 = jnp.bfloat16


SCOPES = False


def _scope(name):
    return jax.named_scope(name) if SCOPES else contextlib.nullcontext()


def _sigmoid(x):
    return 1.0 / (1.0 + jnp.exp(-x))


def _dot_nt(a, b):
    return jax.lax.dot_general(a, b, (((1,), (1,)), ((), ())), preferred_element_type=F32)


def _iota(shape, dim):
    return jax.lax.broadcasted_iota(jnp.int32, shape, dim)


def _kernel(ax_hbm, wqkv_hbm, wo_hbm, wr_ref, wg_hbm, wu_hbm, wd_hbm,
            gw_ref, out_hbm,
            ax_v, wqkv_v, wp_v, wo_v, wop_v, wg_v, wu_v, wd_v,
            qkv_s, o_s, g_s, z_s, out_v, t_s, r_s, xs_v, fence_v,
            sem_ax, sem_w, sem_misc, sem_out, *, S, D):
    DH = D // H
    NS = D // LANES
    NA = S // TM
    qscale = DH ** -0.5 * math.log2(math.e)
    buf_a, buf_b = 0, 3 * NS
    GRP = LANES // H
    UNIT = 2 * LANES

    def ax_copy(i):
        rows = pl.ds(i * TM, TM)
        return pltpu.make_async_copy(ax_hbm.at[rows], ax_v.at[rows], sem_ax.at[i])

    def w_copy(c):
        cols = pl.ds(c * D, D)
        return pltpu.make_async_copy(wqkv_hbm.at[:, cols], wqkv_v.at[c], sem_w.at[c])

    def wq_copy(r0, r1):
        rows = pl.ds(r0, r1 - r0)
        return pltpu.make_async_copy(wqkv_hbm.at[rows, pl.ds(0, D)], wqkv_v.at[0, rows],
                                     sem_w.at[3 + r0 // UNIT])

    wo_copy = pltpu.make_async_copy(wo_hbm, wo_v, sem_misc.at[0])
    wg_copy = pltpu.make_async_copy(wg_hbm, wg_v, sem_misc.at[1])
    wu_copy = pltpu.make_async_copy(wu_hbm, wu_v, sem_misc.at[2])
    wd_copy = pltpu.make_async_copy(wd_hbm, wd_v, sem_misc.at[3])

    fence_copy = pltpu.make_async_copy(ax_hbm.at[pl.ds(0, 16)], fence_v, sem_misc.at[4])

    def out_copy(i):
        rows = pl.ds(OUT_CUTS[i], OUT_CUTS[i + 1] - OUT_CUTS[i])
        return pltpu.make_async_copy(out_v.at[rows], out_hbm.at[rows], sem_out.at[i])

    def permute_unit(pieces):
        w32 = jnp.concatenate(
            [pltpu.bitcast(wqkv_v[c, r0:r0 + nr, :], jnp.int32) for c, r0, nr in pieces], axis=0)
        t_s[...] = w32.T
        for s in range(NS):
            parts = [t_s[pl.ds(s * GRP + j, H, stride=DH), :] for j in range(GRP)]
            blk = jnp.concatenate(parts, axis=0).T
            at = 0
            for c, r0, nr in pieces:
                wp_v[r0 // 2:(r0 + nr) // 2,
                     c * D + s * LANES:c * D + (s + 1) * LANES] = blk[at:at + nr // 2]
                at += nr // 2

    def permute_mxu(c, r0, nr):
        src = _iota((D, D), 0)
        dst = _iota((D, D), 1)
        perm = jnp.where(src == (dst % H) * DH + dst // H, 1.0, 0.0).astype(BF16)
        blk = jnp.dot(wqkv_v[c, r0:r0 + nr, :], perm, preferred_element_type=F32)
        wp_v[r0 // 2:(r0 + nr) // 2, c * D:(c + 1) * D] = pltpu.bitcast(
            blk.astype(BF16), jnp.int32)

    def permute_wo():
        for s in range(NS):
            cols = slice(s * LANES, (s + 1) * LANES)
            t_s[...] = pltpu.bitcast(wo_v[:, cols].astype(F32), jnp.int32)
            for d in range(DH):
                rows = pltpu.bitcast(t_s[pl.ds(d, H, stride=DH), :], F32)
                wop_v[d * H // 2:(d + 1) * H // 2, cols] = pltpu.bitcast(rows.astype(BF16), jnp.int32)

    def project(i, buf, lo, hi):
        x = ax_v[pl.ds(pl.multiple_of(i * TM, TM), TM), :]
        w = pltpu.bitcast(wp_v[:, lo * LANES:hi * LANES], BF16)
        res = jnp.dot(x, w, preferred_element_type=F32)
        for s in range(lo, hi):
            for r0 in range(0, TM, SP):
                piece = res[r0:r0 + SP, (s - lo) * LANES:(s - lo + 1) * LANES]
                if s < NS:
                    piece = piece * qscale
                qkv_s[buf + s, HALO + r0:HALO + r0 + SP, :] = piece
                yield

    def run(gen):
        for _ in gen:
            pass

    def attn_block(i, buf, z):
        row0 = pl.multiple_of(i * TM, TM)
        n = CH

        def shifted(slab, g, w):
            return qkv_s[buf + slab + (z if w >= DYNW else 0),
                         pl.ds(HALO + g - w * DIL, n), :]

        def stage1(g):
            q = [qkv_s[buf + z + s, pl.ds(HALO + g, n), :] for s in range(NS)]
            out = []
            for w in range(WIN):
                p = q[0] * shifted(NS, g, w)
                for s in range(1, NS):
                    p = p + q[s] * shifted(NS + s, g, w)
                out.append((p, pltpu.roll(p, 2 * H, 1)))
            return out

        def stage2(g, st):
            out = []
            for p, pr in st:
                p = p + pr
                out.append((p, pltpu.roll(p, H, 1)))
            return out

        def stage3(g, st):
            logits = []
            for w, (p, pr) in enumerate(st):
                p = p + pr
                if g < w * DIL:
                    pos = row0 + g + _iota((n, LANES), 0)
                    p = jnp.where(pos >= w * DIL, p, -1e9 * math.log2(math.e))
                logits.append(p)
            m = logits[0]
            for w in range(1, WIN):
                m = jnp.maximum(m, logits[w])
            e = [jnp.exp2(l - m) for l in logits]
            den = e[0]
            for w in range(1, WIN):
                den = den + e[w]
            inv = 1.0 / den
            out = []
            for s in range(NS):
                acc = e[0] * shifted(2 * NS + s, g, 0)
                for w in range(1, WIN):
                    acc = acc + e[w] * shifted(2 * NS + s, g, w)
                out.append(acc * inv)
            return out

        groups = list(range(0, TM, n))
        s1, s2, pend = {}, {}, []
        for t in range(len(groups) + 2):
            if t < len(groups):
                s1[t] = stage1(groups[t])
            if 0 <= t - 1 < len(groups):
                s2[t - 1] = stage2(groups[t - 1], s1.pop(t - 1))
            if 0 <= t - 2 < len(groups):
                pend.append(stage3(groups[t - 2], s2.pop(t - 2)))
                if len(pend) * n >= 16:
                    g0 = groups[t - 2] + n - len(pend) * n
                    for s in range(NS):
                        o = jnp.concatenate([p[s] for p in pend], axis=0)
                        o_s[pl.ds(pl.multiple_of((row0 + g0) // 2, 8), len(pend) * n // 2),
                            s * LANES:(s + 1) * LANES] = pltpu.bitcast(o.astype(BF16), jnp.int32)
                    pend = []
            yield

    def row_dot(x, which):
        p = None
        for s in range(NS):
            w = qkv_s[6 * NS, pl.ds(pl.multiple_of((which + s) * 16, 16), 16), :]
            t = x[:, s * LANES:(s + 1) * LANES] * w
            p = t if p is None else p + t
        return jnp.sum(p, axis=1, keepdims=True)

    def route_block(i, z):
        lane = _iota((8, LANES), 1)
        acc = jnp.full((8, LANES), -jnp.inf, F32)
        for g in range(0, TM, 16):
            rows = pl.ds(pl.multiple_of(i * TM + g, 16), 16)
            x = ax_v[rows, :].astype(F32)
            r = row_dot(x, z)
            acc = jnp.where(lane == g // 8, r[:8], acc)
            acc = jnp.where(lane == g // 8 + 1, r[8:], acc)
            g_s[rows, :] = jnp.broadcast_to(_sigmoid(row_dot(x, z + NS)), (16, LANES))
            if g + 16 == TM:
                r_s[pl.ds(pl.multiple_of(i * 8, 8), 8), :] = acc
            yield

    wq_cuts = list(range(0, D, UNIT)) + [D]
    wq_parts = list(zip(wq_cuts[:-1], wq_cuts[1:]))
    for part in (2, 0, 1):
        wq_copy(*wq_parts[part]).start()
    z_s[0] = 0
    for n, ref in enumerate((wr_ref, gw_ref)):
        w = ref[...].astype(F32).reshape(1, D)
        for s in range(NS):
            qkv_s[6 * NS, (n * NS + s) * 16:(n * NS + s + 1) * 16, :] = jnp.broadcast_to(
                w[:, s * LANES:(s + 1) * LANES], (16, LANES))
    tail0, tail = wq_parts[-1][0], D - wq_parts[-1][0]
    with _scope("perm0"):
        wq_copy(*wq_parts[2]).wait()
        wq_copy(*wq_parts[0]).wait()
        ax_copy(0).start()
        permute_mxu(0, tail0, tail)
        permute_unit([(0, 0, UNIT)])
        wq_copy(*wq_parts[1]).wait()
        w_copy(1).start()
        ax_copy(1).start()
        permute_unit([(0, UNIT, UNIT)])
    with _scope("q0"):
        ax_copy(0).wait()
        w_copy(2).start()
        run(project(0, buf_a, 0, NS))
        run(route_block(0, 0))
    with _scope("q1"):
        w_copy(1).wait()
        ax_copy(1).wait()
        for i in range(2, NA):
            ax_copy(i).start()
        run(project(1, buf_b, 0, NS))
        permute_unit([(1, 0, UNIT)])
        permute_unit([(1, UNIT, UNIT)])
        permute_unit([(1, tail0, tail), (1, tail0, tail)])
    with _scope("kv0"):
        w_copy(2).wait()
        ax_copy(2).wait()
        wg_copy.start()
        wu_copy.start()
        wd_copy.start()
        wo_copy.start()
        fence_copy.start()
        run(project(0, buf_a, NS, 2 * NS))
        permute_unit([(2, 0, UNIT)])
        permute_unit([(2, UNIT, UNIT)])
        permute_unit([(2, tail0, tail), (2, tail0, tail)])
        run(project(0, buf_a, 2 * NS, 3 * NS))
        run(route_block(1, 0))
        for s in range(NS, 3 * NS):
            qkv_s[s, 0:HALO, :] = jnp.broadcast_to(qkv_s[s, HALO:HALO + 1, :], (HALO, LANES))

    def step_a(i, src, dst, first=False, last=False):
        for s in range(NS, 3 * NS):
            qkv_s[dst + s, 0:HALO, :] = qkv_s[src + s, TM:TM + HALO, :]
        z = z_s[0]
        jobs = [[attn_block(i - 1, src, z), TM // CH + 2, 0]]
        if not last:
            jobs.append([route_block(i + 1, z), TM // 16, 0])
        lo = NS if first else 0
        n_mm = (3 * NS - lo) * (TM // SP)
        k = 0
        for _ in project(i, dst, lo, 3 * NS):
            k += 1
            for job in jobs:
                upto = min(job[1], max(0, round((k - LAG) * job[1] / (n_mm - LAG - LEAD))))
                for _ in range(upto - job[2]):
                    next(job[0])
                job[2] = upto

    def body_a(j, carry):
        i = 2 * j + 2
        ax_copy(i + 1).wait()
        ax_copy(i + 2).wait()
        step_a(i, buf_b, buf_a)
        step_a(i + 1, buf_a, buf_b)
        return carry

    with _scope("step1"):
        step_a(1, buf_a, buf_b, first=True)
    with _scope("loopA"):
        jax.lax.fori_loop(0, (NA - 4) // 2, body_a, 0)
    ax_copy(NA - 1).wait()
    wo_copy.wait()
    step_a(NA - 2 + z_s[0], buf_b, buf_a)

    nr = NA * 8
    r = r_s[...].astype(BF16).astype(F32)
    r = jnp.where(r != r, -jnp.inf, r)
    sub = _iota((nr, LANES), 0)
    col = _iota((nr, LANES), 1)
    tok = jnp.where(col < TM // 8, (sub // 8) * TM + col * 8 + sub % 8, S - 1)
    m1 = jnp.max(r)
    i1 = jnp.min(jnp.where(r == m1, tok, S - 1))
    r2 = jnp.where(tok == i1, -jnp.inf, r)
    m2 = jnp.max(r2)
    i2 = jnp.min(jnp.where((r2 == m2) & (tok != i1), tok, S - 1))

    row16 = _iota((16, D), 0)

    def tile_of(i):
        return pl.ds(pl.multiple_of((i // 16) * 16, 16), 16)

    def pick(i):
        tile = ax_v[tile_of(i), :].astype(F32)
        return jnp.sum(jnp.where(row16 == i % 16, tile, 0.0), axis=0, keepdims=True)

    xsel = jnp.where(row16 == 0, pick(i1), jnp.where(row16 == 1, pick(i2), 0.0))
    xsel = xsel.astype(BF16)
    xs_v[...] = xsel
    permute_wo()
    step_a(NA - 1 + z_s[0], buf_a, buf_b, last=True)
    wg_copy.wait()
    wu_copy.wait()
    wd_copy.wait()
    gg = _dot_nt(xs_v[...], wg_v[...])
    uu = _dot_nt(xs_v[...], wu_v[...])
    hh = (gg * _sigmoid(gg) * uu).astype(BF16)
    y = jnp.dot(hh, wd_v[...], preferred_element_type=F32)
    run(attn_block(NA - 1, buf_b, 0))
    for n, (i, m) in enumerate(((i1, m1), (i2, m2))):
        upd = y[n:n + 1, :] * _sigmoid(jnp.full((1, D), m, F32))
        tile = ax_v[tile_of(i), :].astype(F32)
        ax_v[tile_of(i), :] = jnp.where(row16 == i % 16, tile + upd, tile).astype(BF16)

    def out_rows(t):
        row0, row1 = OUT_CUTS[t], OUT_CUTS[t + 1]
        o = pltpu.bitcast(o_s[row0 // 2:row1 // 2, :], BF16)
        a = jnp.dot(o, pltpu.bitcast(wop_v[...], BF16), preferred_element_type=F32)
        g = g_s[row0:row1, :]
        for s in range(NS):
            cols = slice(s * LANES, (s + 1) * LANES)
            b = ax_v[row0:row1, cols].astype(F32)
            out_v[row0:row1, cols] = (g * a[:, cols] + (1.0 - g) * b).astype(BF16)
        out_copy(t).start()

    for t in range(len(OUT_CUTS) - 1):
        if t == FENCE:
            fence_copy.wait()
        out_rows(t)
    with _scope("drain"):
        for t in range(len(OUT_CUTS) - 1):
            out_copy(t).wait()


@jax.jit
def pallas_gated_mix__sliding_local_dilated__moe_arch_mod__prompt_kernel(
    A_x: jax.Array,
    A_wqkv: jax.Array,
    A_wo: jax.Array,
    B_x: jax.Array,
    B_w_r: jax.Array,
    B_w_gate: jax.Array,
    B_w_up: jax.Array,
    B_w_down: jax.Array,
    gate_w: jax.Array,
):
    B, S, D = A_x.shape
    F = B_w_gate.shape[1]
    assert B == 1
    NS = D // LANES
    hbm = pl.BlockSpec(memory_space=pltpu.HBM)
    vmem = pl.BlockSpec(memory_space=pltpu.VMEM)
    out = pl.pallas_call(
        functools.partial(_kernel, S=S, D=D),
        out_shape=jax.ShapeDtypeStruct((S, D), A_x.dtype),
        in_specs=[hbm, hbm, hbm, vmem, hbm, hbm, hbm, vmem],
        out_specs=hbm,
        scratch_shapes=[
            pltpu.VMEM((S, D), BF16),
            pltpu.VMEM((3, D, D), BF16),
            pltpu.VMEM((D // 2, 3 * D), jnp.int32),
            pltpu.VMEM((D, D), BF16),
            pltpu.VMEM((D // 2, D), jnp.int32),
            pltpu.VMEM((F, D), BF16),
            pltpu.VMEM((F, D), BF16),
            pltpu.VMEM((F, D), BF16),
            pltpu.VMEM((6 * NS + 1, HALO + TM, LANES), F32),
            pltpu.VMEM((S // 2, D), jnp.int32),
            pltpu.VMEM((S, LANES), F32),
            pltpu.SMEM((1,), jnp.int32),
            pltpu.VMEM((S, D), BF16),
            pltpu.VMEM((D, LANES), jnp.int32),
            pltpu.VMEM((S // TM * 8, LANES), F32),
            pltpu.VMEM((16, D), BF16),
            pltpu.VMEM((16, D), BF16),
            pltpu.SemaphoreType.DMA((S // TM,)),
            pltpu.SemaphoreType.DMA((6,)),
            pltpu.SemaphoreType.DMA((5,)),
            pltpu.SemaphoreType.DMA((len(OUT_CUTS) - 1,)),
        ],
        compiler_params=pltpu.CompilerParams(vmem_limit_bytes=100 * 2**20, flags=FLAGS),
    )(A_x.reshape(S, D), A_wqkv, A_wo, B_w_r,
      B_w_gate.T, B_w_up.T, B_w_down, gate_w)
    return out.reshape(B, S, D)
```

```python
import contextlib
import functools
import math

import jax
import jax.numpy as jnp
import numpy as np
from jax.experimental import pallas as pl
from jax.experimental.pallas import tpu as pltpu

H = 32
WIN = 8
DIL = 2
HALO = 16
LANES = 128
TM = 256
OUT_CUTS = (0, 256, 512, 768, 1024, 1280, 1536, 1792, 1920, 1984, 2048)
FENCE = 3
NMXU = 4
SKIP = 3
TR = 128
LEADF = 16
FLAGS = {}
SP = 16
LAG = 0
LEAD = 3
DYNW = 7
CH = 8
F32 = jnp.float32
BF16 = jnp.bfloat16


SCOPES = False


def _scope(name):
    return jax.named_scope(name) if SCOPES else contextlib.nullcontext()


def _sigmoid(x):
    return 1.0 / (1.0 + jnp.exp(-x))


def _dot_nt(a, b):
    return jax.lax.dot_general(a, b, (((1,), (1,)), ((), ())), preferred_element_type=F32)


def _iota(shape, dim):
    return jax.lax.broadcasted_iota(jnp.int32, shape, dim)


def _kernel(ax_hbm, wqkv_hbm, wo_hbm, wr_ref, wg_hbm, wu_hbm, wd_hbm,
            gw_ref, out_hbm,
            ax_v, wqkv_v, wp_v, wo_v, wop_v, wg_v, wu_v, wd_v,
            qkv_s, o_s, g_s, z_s, out_v, t_s, two_s, r_s, hs_v, fence_v,
            sem_ax, sem_w, sem_misc, sem_out, *, S, D, F):
    DH = D // H
    NS = D // LANES
    NA = S // TM
    qscale = DH ** -0.5 * math.log2(math.e)
    buf_a, buf_b = 0, 3 * NS
    RPB = TM // TR
    RPS = (NA - 2) * RPB // (NA - 4)
    GRP = LANES // H
    UNIT = 2 * LANES

    def ax_copy(i):
        rows = pl.ds(i * TM, TM)
        return pltpu.make_async_copy(ax_hbm.at[rows], ax_v.at[rows], sem_ax.at[i])

    def w_copy(c):
        cols = pl.ds(c * D, D)
        return pltpu.make_async_copy(wqkv_hbm.at[:, cols], wqkv_v.at[c], sem_w.at[c])

    def wq_copy(r0, r1):
        rows = pl.ds(r0, r1 - r0)
        return pltpu.make_async_copy(wqkv_hbm.at[rows, pl.ds(0, D)], wqkv_v.at[0, rows],
                                     sem_w.at[3 + r0 // UNIT])

    wo_copy = pltpu.make_async_copy(wo_hbm, wo_v, sem_misc.at[0])
    wg_copy = pltpu.make_async_copy(wg_hbm, wg_v, sem_misc.at[1])
    wu_copy = pltpu.make_async_copy(wu_hbm, wu_v, sem_misc.at[2])
    wd_copy = pltpu.make_async_copy(wd_hbm, wd_v, sem_misc.at[3])

    def fence_copy(n):
        return pltpu.make_async_copy(ax_hbm.at[pl.ds(0, 16)], fence_v.at[n], sem_misc.at[4 + n])

    def out_copy(i):
        rows = pl.ds(OUT_CUTS[i], OUT_CUTS[i + 1] - OUT_CUTS[i])
        return pltpu.make_async_copy(out_v.at[rows], out_hbm.at[rows], sem_out.at[i])

    units = [0]

    def permute_unit(pieces):
        w32 = jnp.concatenate(
            [pltpu.bitcast(wqkv_v[c, r0:r0 + nr, :], jnp.int32) for c, r0, nr in pieces], axis=0)
        tb = units[0] % 2
        units[0] += 1
        t_s[tb] = w32.T
        for s in range(NS):
            parts = [t_s[tb, pl.ds(s * GRP + j, H, stride=DH), :] for j in range(GRP)]
            blk = jnp.concatenate(parts, axis=0).T
            at = 0
            for c, r0, nr in pieces:
                wp_v[r0 // 2:(r0 + nr) // 2,
                     c * D + s * LANES:c * D + (s + 1) * LANES] = blk[at:at + nr // 2]
                at += nr // 2

    def permute_mxu(c, r0, nr):
        blk = jnp.dot(wqkv_v[c, r0:r0 + nr, :], pltpu.bitcast(wop_v[...], BF16),
                      preferred_element_type=F32)
        wp_v[r0 // 2:(r0 + nr) // 2, c * D:(c + 1) * D] = pltpu.bitcast(
            blk.astype(BF16), jnp.int32)

    def permute_wo():
        for s in range(NS):
            cols = slice(s * LANES, (s + 1) * LANES)
            two_s[s] = wo_v[:, cols].astype(F32)
            for d in range(DH):
                rows = two_s[s, pl.ds(d, H, stride=DH), :]
                wop_v[d * H // 2:(d + 1) * H // 2, cols] = pltpu.bitcast(
                    rows.astype(BF16), jnp.int32)

    def project(i, buf, lo, hi, filler=None):
        rows = pl.ds(pl.multiple_of(i * TM, TM), TM)

        def product(k0, k1, c0, c1):
            w = pltpu.bitcast(wp_v[k0 // 2:k1 // 2, c0 * LANES:c1 * LANES], BF16)
            res = jnp.dot(ax_v[rows, k0:k1], w, preferred_element_type=F32)
            if filler is not None:
                next(filler, None)
            return res

        width = hi - lo if filler is None else NMXU
        split = 0 if filler is None else NMXU * LANES
        for c0 in range(lo, hi, width):
            c1 = min(c0 + width, hi)
            rest = product(split, D, c0, c1)
            for s in range(c0, c1):
                res = rest[:, (s - c0) * LANES:(s - c0 + 1) * LANES]
                if split:
                    res = res + product(0, split, s, s + 1)
                if s < NS:
                    res = res * qscale
                for r0 in range(0, TM, SP):
                    qkv_s[buf + s, HALO + r0:HALO + r0 + SP, :] = res[r0:r0 + SP]
                    yield

    def run(gen):
        for _ in gen:
            pass

    def attn_block(i, buf, z):
        row0 = pl.multiple_of(i * TM, TM)
        n = CH

        def shifted(slab, g, w):
            return qkv_s[buf + slab + (z if w >= DYNW else 0),
                         pl.ds(HALO + g - w * DIL, n), :]

        def stage1(g):
            q = [qkv_s[buf + z + s, pl.ds(HALO + g, n), :] for s in range(NS)]
            out = []
            for w in range(WIN):
                p = q[0] * shifted(NS, g, w)
                for s in range(1, NS):
                    p = p + q[s] * shifted(NS + s, g, w)
                out.append((p, pltpu.roll(p, 2 * H, 1)))
            return out

        def stage2(g, st):
            out = []
            for p, pr in st:
                p = p + pr
                out.append((p, pltpu.roll(p, H, 1)))
            return out

        def stage3(g, st):
            logits = []
            for w, (p, pr) in enumerate(st):
                p = p + pr
                if g < w * DIL:
                    pos = row0 + g + _iota((n, LANES), 0)
                    p = jnp.where(pos >= w * DIL, p, -1e9 * math.log2(math.e))
                logits.append(p)
            m = logits[0]
            for w in range(1, WIN):
                m = jnp.maximum(m, logits[w])
            e = [jnp.exp2(l - m) for l in logits]
            den = e[0]
            for w in range(1, WIN):
                den = den + e[w]
            inv = 1.0 / den
            out = []
            for s in range(NS):
                acc = e[0] * shifted(2 * NS + s, g, 0)
                for w in range(1, WIN):
                    acc = acc + e[w] * shifted(2 * NS + s, g, w)
                out.append(acc * inv)
            return out

        groups = list(range(0, TM, n))
        s1, s2, pend = {}, {}, []
        for t in range(len(groups) + 2):
            if t < len(groups):
                s1[t] = stage1(groups[t])
            if 0 <= t - 1 < len(groups):
                s2[t - 1] = stage2(groups[t - 1], s1.pop(t - 1))
            if 0 <= t - 2 < len(groups):
                pend.append(stage3(groups[t - 2], s2.pop(t - 2)))
                if len(pend) * n >= 16:
                    g0 = groups[t - 2] + n - len(pend) * n
                    for s in range(NS):
                        o = jnp.concatenate([p[s] for p in pend], axis=0)
                        o_s[pl.ds(pl.multiple_of((row0 + g0) // 2, 8), len(pend) * n // 2),
                            s * LANES:(s + 1) * LANES] = pltpu.bitcast(o.astype(BF16), jnp.int32)
                    pend = []
            yield

    def row_dot(x, which):
        p = None
        for s in range(NS):
            w = qkv_s[6 * NS, pl.ds(pl.multiple_of((which + s) * 16, 16), 16), :]
            t = x[:, s * LANES:(s + 1) * LANES] * w
            p = t if p is None else p + t
        return jnp.sum(p, axis=1, keepdims=True)

    def route(first, count, z):
        lane = _iota((8, LANES), 1)
        for i in range(count):
            acc = jnp.full((8, LANES), -jnp.inf, F32)
            for g in range(0, TR, 16):
                rows = pl.ds(pl.multiple_of((first + i) * TR + g, 16), 16)
                x = ax_v[rows, :].astype(F32)
                r = row_dot(x, z)
                acc = jnp.where(lane == g // 8, r[:8], acc)
                acc = jnp.where(lane == g // 8 + 1, r[8:], acc)
                g_s[rows, :] = jnp.broadcast_to(_sigmoid(row_dot(x, z + NS)), (16, LANES))
                if g + 16 == TR:
                    r_s[pl.ds(pl.multiple_of((first + i) * 8, 8), 8), :] = acc
                yield

    wq_cuts = list(range(0, D, UNIT)) + [D]
    wq_parts = list(zip(wq_cuts[:-1], wq_cuts[1:]))
    wq_copy(*wq_parts[0]).start()
    z_s[0] = 0
    for n, ref in enumerate((wr_ref, gw_ref)):
        w = ref[...].astype(F32).reshape(1, D)
        for s in range(NS):
            qkv_s[6 * NS, (n * NS + s) * 16:(n * NS + s + 1) * 16, :] = jnp.broadcast_to(
                w[:, s * LANES:(s + 1) * LANES], (16, LANES))
    tail0, tail = wq_parts[-1][0], D - wq_parts[-1][0]
    dst_col = _iota((D, D), 1)
    perm = jnp.where(_iota((D, D), 0) == (dst_col % H) * DH + dst_col // H, 1.0, 0.0)
    wop_v[...] = pltpu.bitcast(perm.astype(BF16), jnp.int32)
    for part in wq_parts[1:]:
        wq_copy(*part).start()
    with _scope("perm0"):
        wq_copy(*wq_parts[0]).wait()
        ax_copy(0).start()
        permute_unit([(0, 0, UNIT)])
        for part in wq_parts[1:]:
            wq_copy(*part).wait()
        w_copy(1).start()
        permute_mxu(0, tail0, tail)
        permute_unit([(0, UNIT, UNIT)])
    with _scope("w_q0"):
        ax_copy(0).wait()
    with _scope("q0"):
        ax_copy(1).start()
        w_copy(2).start()
        run(project(0, buf_a, 0, NS))
        run(route(0, RPB, 0))
    with _scope("w_q1"):
        w_copy(1).wait()
        ax_copy(1).wait()
    with _scope("q1"):
        ax_copy(2).start()
        ax_copy(3).start()
        run(project(1, buf_b, 0, NS))
        permute_unit([(1, 0, UNIT)])
        permute_unit([(1, UNIT, UNIT)])
        permute_unit([(1, tail0, tail), (1, tail0, tail)])
    with _scope("w_kv0"):
        w_copy(2).wait()
    with _scope("kv0"):
        for i in range(4, NA):
            ax_copy(i).start()
        wg_copy.start()
        wu_copy.start()
        wd_copy.start()
        wo_copy.start()
        fence_copy(0).start()
        fence_copy(1).start()
        run(project(0, buf_a, NS, 2 * NS))
        permute_unit([(2, 0, UNIT)])
        permute_unit([(2, UNIT, UNIT)])
        permute_unit([(2, tail0, tail), (2, tail0, tail)])
        run(project(0, buf_a, 2 * NS, 3 * NS))
        run(route(RPB, RPB, 0))
        for s in range(NS, 3 * NS):
            qkv_s[s, 0:HALO, :] = jnp.broadcast_to(qkv_s[s, HALO:HALO + 1, :], (HALO, LANES))

    def step_a(i, src, dst, first=False, filler=None):
        for s in range(NS, 3 * NS):
            qkv_s[dst + s, 0:HALO, :] = qkv_s[src + s, TM:TM + HALO, :]
        z = z_s[0]
        jobs = [[attn_block(i - 1, src, z), TM // CH + 2, 0]]
        if filler is None and not first:
            jobs.append([route(2 * RPB + (i - 2) * RPS, RPS, z), RPS * TR // 16, 0])
        lo = NS if first else 0
        n_mm = (3 * NS - lo) * (TM // SP)
        k, lead = 0, (LEAD if filler is None else LEADF)
        for _ in project(i, dst, lo, 3 * NS, filler):
            k += 1
            for job in jobs:
                upto = min(job[1], max(0, round((k - LAG) * job[1] / (n_mm - LAG - lead))))
                for _ in range(upto - job[2]):
                    next(job[0])
                job[2] = upto

    def body_a(j, carry):
        i = 2 * j + 2
        for n in range(2 * RPS // RPB):
            ax_copy(2 + j * (2 * RPS // RPB) + n).wait()
        step_a(i, buf_b, buf_a)
        step_a(i + 1, buf_a, buf_b)
        return carry

    with _scope("step1"):
        step_a(1 + z_s[0], buf_a, buf_b, first=True)
    with _scope("loopA"):
        jax.lax.fori_loop(0, (NA - 4) // 2, body_a, 0)
    wo_copy.wait()
    wg_copy.wait()
    wu_copy.wait()
    wd_copy.wait()

    nr = S // TR * 8
    r = r_s[...].astype(BF16).astype(F32)
    r = jnp.where(r != r, -jnp.inf, r)
    sub = _iota((nr, LANES), 0)
    col = _iota((nr, LANES), 1)
    tok = jnp.where(col < TR // 8, (sub // 8) * TR + col * 8 + sub % 8, S - 1)
    m1 = jnp.max(r)
    i1 = jnp.min(jnp.where(r == m1, tok, S - 1))
    r2 = jnp.where(tok == i1, -jnp.inf, r)
    m2 = jnp.max(r2)
    i2 = jnp.min(jnp.where((r2 == m2) & (tok != i1), tok, S - 1))

    row16 = _iota((16, D), 0)

    def tile_of(i):
        return pl.ds(pl.multiple_of((i // 16) * 16, 16), 16)

    def pick(i):
        tile = ax_v[tile_of(i), :].astype(F32)
        return jnp.sum(jnp.where(row16 == i % 16, tile, 0.0), axis=0, keepdims=True)

    xsel = jnp.where(row16 == 0, pick(i1), jnp.where(row16 == 1, pick(i2), 0.0))
    xsel = xsel.astype(BF16)
    hidden = []

    def ffn_up():
        for _ in range(SKIP):
            yield
        n = NMXU * LANES
        for f0 in range(0, F, n):
            nf = min(n, F - f0)
            if 2 * nf <= n:
                operands = [lambda ks: jnp.concatenate(
                    [wg_v[f0:f0 + nf, ks], wu_v[f0:f0 + nf, ks]], axis=0)]
            else:
                operands = [lambda ks: wg_v[f0:f0 + nf, ks], lambda ks: wu_v[f0:f0 + nf, ks]]
            accs = []
            for operand in operands:
                acc = None
                for k0 in range(0, D, LANES):
                    ks = slice(k0, k0 + LANES)
                    part = _dot_nt(xsel[:, ks], operand(ks))
                    acc = part if acc is None else acc + part
                    yield
                accs.append(acc)
            gg, uu = accs if len(accs) == 2 else (accs[0][:, :nf], accs[0][:, nf:])
            hidden.append((gg * _sigmoid(gg) * uu).astype(BF16))

    filler = ffn_up()
    step_a(NA - 2 + z_s[0], buf_b, buf_a, filler=filler)
    step_a(NA - 1 + z_s[0], buf_a, buf_b, filler=filler)
    run(filler)
    hs_v[...] = jnp.concatenate(hidden, axis=1)
    fence_copy(0).wait()
    permute_wo()
    y = jnp.dot(hs_v[...], wd_v[...], preferred_element_type=F32)
    run(attn_block(NA - 1, buf_b, 0))
    for n, (i, m) in enumerate(((i1, m1), (i2, m2))):
        upd = y[n:n + 1, :] * _sigmoid(jnp.full((1, D), m, F32))
        tile = ax_v[tile_of(i), :].astype(F32)
        ax_v[tile_of(i), :] = jnp.where(row16 == i % 16, tile + upd, tile).astype(BF16)

    def out_rows(t):
        row0, row1 = OUT_CUTS[t], OUT_CUTS[t + 1]
        o = pltpu.bitcast(o_s[row0 // 2:row1 // 2, :], BF16)
        a = jnp.dot(o, pltpu.bitcast(wop_v[...], BF16), preferred_element_type=F32)
        g = g_s[row0:row1, :]
        for s in range(NS):
            cols = slice(s * LANES, (s + 1) * LANES)
            b = ax_v[row0:row1, cols].astype(F32)
            out_v[row0:row1, cols] = (g * a[:, cols] + (1.0 - g) * b).astype(BF16)
        out_copy(t).start()

    for t in range(len(OUT_CUTS) - 1):
        if t == FENCE:
            fence_copy(1).wait()
        out_rows(t)
    with _scope("drain"):
        for t in range(len(OUT_CUTS) - 1):
            out_copy(t).wait()


@jax.jit
def pallas_gated_mix__sliding_local_dilated__moe_arch_mod__prompt_kernel(
    A_x: jax.Array,
    A_wqkv: jax.Array,
    A_wo: jax.Array,
    B_x: jax.Array,
    B_w_r: jax.Array,
    B_w_gate: jax.Array,
    B_w_up: jax.Array,
    B_w_down: jax.Array,
    gate_w: jax.Array,
):
    B, S, D = A_x.shape
    F = B_w_gate.shape[1]
    assert B == 1
    NS = D // LANES
    hbm = pl.BlockSpec(memory_space=pltpu.HBM)
    vmem = pl.BlockSpec(memory_space=pltpu.VMEM)
    out = pl.pallas_call(
        functools.partial(_kernel, S=S, D=D, F=F),
        out_shape=jax.ShapeDtypeStruct((S, D), A_x.dtype),
        in_specs=[hbm, hbm, hbm, vmem, hbm, hbm, hbm, vmem],
        out_specs=hbm,
        scratch_shapes=[
            pltpu.VMEM((S, D), BF16),
            pltpu.VMEM((3, D, D), BF16),
            pltpu.VMEM((D // 2, 3 * D), jnp.int32),
            pltpu.VMEM((D, D), BF16),
            pltpu.VMEM((D // 2, D), jnp.int32),
            pltpu.VMEM((F, D), BF16),
            pltpu.VMEM((F, D), BF16),
            pltpu.VMEM((F, D), BF16),
            pltpu.VMEM((6 * NS + 1, HALO + TM, LANES), F32),
            pltpu.VMEM((S // 2, D), jnp.int32),
            pltpu.VMEM((S, LANES), F32),
            pltpu.SMEM((1,), jnp.int32),
            pltpu.VMEM((S, D), BF16),
            pltpu.VMEM((2, D, LANES), jnp.int32),
            pltpu.VMEM((NS, D, LANES), F32),
            pltpu.VMEM((S // TR * 8, LANES), F32),
            pltpu.VMEM((16, F), BF16),
            pltpu.VMEM((2, 16, D), BF16),
            pltpu.SemaphoreType.DMA((S // TM,)),
            pltpu.SemaphoreType.DMA((6,)),
            pltpu.SemaphoreType.DMA((6,)),
            pltpu.SemaphoreType.DMA((len(OUT_CUTS) - 1,)),
        ],
        compiler_params=pltpu.CompilerParams(vmem_limit_bytes=100 * 2**20, flags=FLAGS),
    )(A_x.reshape(S, D), A_wqkv, A_wo, B_w_r,
      B_w_gate.T, B_w_up.T, B_w_down, gate_w)
    return out.reshape(B, S, D)
```

```python
import contextlib
import functools
import math

import jax
import jax.numpy as jnp
import numpy as np
from jax.experimental import pallas as pl
from jax.experimental.pallas import tpu as pltpu

H = 32
WIN = 8
DIL = 2
HALO = 16
LANES = 128
TM = 256
OUT_CUTS = (0, 256, 512, 768, 1024, 1280, 1536, 1792, 1920, 1984, 2048)
SPREAD = 5
NMXU = 4
SKIP = 4
SPC = 64
CLAG = -1
CLEAD = 1
TR = 128
LEADF = 16
FLAGS = {}
SP = 16
LAG = 0
LEAD = 3
DYNW = 8
CH = 8
F32 = jnp.float32
BF16 = jnp.bfloat16


SCOPES = False


def _scope(name):
    return jax.named_scope(name) if SCOPES else contextlib.nullcontext()


def _sigmoid(x):
    return 0.5 * jnp.tanh(0.5 * x) + 0.5


def _dot_nt(a, b):
    return jax.lax.dot_general(a, b, (((1,), (1,)), ((), ())), preferred_element_type=F32)


def _iota(shape, dim):
    return jax.lax.broadcasted_iota(jnp.int32, shape, dim)


def _kernel(ax_hbm, wqkv_hbm, wo_hbm, wr_ref, wg_hbm, wu_hbm, wd_hbm,
            gw_ref, out_hbm,
            ax_v, wqkv_v, wp_v, wo_v, wop_v, wg_v, wu_v, wd_v,
            qkv_s, o_s, g_s, z_s, out_v, t_s, two_s, r_s, hs_v, fence_v,
            sem_ax, sem_w, sem_misc, sem_out, *, S, D, F):
    DH = D // H
    NS = D // LANES
    NA = S // TM
    qscale = DH ** -0.5 * math.log2(math.e)
    buf_a, buf_b = 0, 3 * NS
    RPB = TM // TR
    RPS = (NA - 2) * RPB // (NA - 4)
    GRP = LANES // H
    UNIT = 2 * LANES

    def ax_copy(i):
        rows = pl.ds(i * TM, TM)
        return pltpu.make_async_copy(ax_hbm.at[rows], ax_v.at[rows], sem_ax.at[i])

    def w_copy(c):
        cols = pl.ds(c * D, D)
        return pltpu.make_async_copy(wqkv_hbm.at[:, cols], wqkv_v.at[c], sem_w.at[c])

    def wq_copy(r0, r1):
        rows = pl.ds(r0, r1 - r0)
        return pltpu.make_async_copy(wqkv_hbm.at[rows, pl.ds(0, D)], wqkv_v.at[0, rows],
                                     sem_w.at[3 + r0 // UNIT])

    wo_copy = pltpu.make_async_copy(wo_hbm, wo_v, sem_misc.at[0])
    wg_copy = pltpu.make_async_copy(wg_hbm, wg_v, sem_misc.at[1])
    wu_copy = pltpu.make_async_copy(wu_hbm, wu_v, sem_misc.at[2])
    wd_copy = pltpu.make_async_copy(wd_hbm, wd_v, sem_misc.at[3])

    fence_copy = pltpu.make_async_copy(ax_hbm.at[pl.ds(0, 16)], fence_v, sem_misc.at[4])

    def out_copy(i):
        rows = pl.ds(OUT_CUTS[i], OUT_CUTS[i + 1] - OUT_CUTS[i])
        return pltpu.make_async_copy(out_v.at[rows], out_hbm.at[rows], sem_out.at[i])

    units = [0]

    def permute_unit(pieces):
        w32 = jnp.concatenate(
            [pltpu.bitcast(wqkv_v[c, r0:r0 + nr, :], jnp.int32) for c, r0, nr in pieces], axis=0)
        tb = units[0] % 2
        units[0] += 1
        t_s[tb] = w32.T
        for s in range(NS):
            parts = [t_s[tb, pl.ds(s * GRP + j, H, stride=DH), :] for j in range(GRP)]
            blk = jnp.concatenate(parts, axis=0).T
            at = 0
            for c, r0, nr in pieces:
                wp_v[r0 // 2:(r0 + nr) // 2,
                     c * D + s * LANES:c * D + (s + 1) * LANES] = blk[at:at + nr // 2]
                at += nr // 2

    def permute_mxu(c, r0, nr):
        blk = jnp.dot(wqkv_v[c, r0:r0 + nr, :], pltpu.bitcast(wop_v[...], BF16),
                      preferred_element_type=F32)
        wp_v[r0 // 2:(r0 + nr) // 2, c * D:(c + 1) * D] = pltpu.bitcast(
            blk.astype(BF16), jnp.int32)

    def permute_wo():
        for s in range(NS):
            cols = slice(s * LANES, (s + 1) * LANES)
            two_s[s] = wo_v[:, cols].astype(F32)
            for d in range(DH):
                rows = two_s[s, pl.ds(d, H, stride=DH), :]
                wop_v[d * H // 2:(d + 1) * H // 2, cols] = pltpu.bitcast(
                    rows.astype(BF16), jnp.int32)

    def project(i, buf, lo, hi, filler=None):
        rows = pl.ds(pl.multiple_of(i * TM, TM), TM)

        def product(k0, k1, c0, c1):
            w = pltpu.bitcast(wp_v[k0 // 2:k1 // 2, c0 * LANES:c1 * LANES], BF16)
            res = jnp.dot(ax_v[rows, k0:k1], w, preferred_element_type=F32)
            if filler is not None:
                next(filler, None)
            return res

        width = hi - lo if filler is None else NMXU
        split = 0 if filler is None else NMXU * LANES
        for c0 in range(lo, hi, width):
            c1 = min(c0 + width, hi)
            rest = product(split, D, c0, c1)
            for s in range(c0, c1):
                res = rest[:, (s - c0) * LANES:(s - c0 + 1) * LANES]
                if split:
                    res = res + product(0, split, s, s + 1)
                if s < NS:
                    res = res * qscale
                for r0 in range(0, TM, SP):
                    qkv_s[buf + s, HALO + r0:HALO + r0 + SP, :] = res[r0:r0 + SP]
                    yield

    def run(gen):
        for _ in gen:
            pass

    def attn_block(i, buf, z):
        row0 = pl.multiple_of(i * TM, TM)
        n = CH

        def shifted(slab, g, w):
            return qkv_s[buf + slab + (z if w >= DYNW else 0),
                         pl.ds(HALO + g - w * DIL, n), :]

        def stage1(g):
            q = [qkv_s[buf + z + s, pl.ds(HALO + g, n), :] for s in range(NS)]
            out = []
            for w in range(WIN):
                p = q[0] * shifted(NS, g, w)
                for s in range(1, NS):
                    p = p + q[s] * shifted(NS + s, g, w)
                out.append((p, pltpu.roll(p, 2 * H, 1)))
            return out

        def stage2(g, st):
            out = []
            for p, pr in st:
                p = p + pr
                out.append((p, pltpu.roll(p, H, 1)))
            return out

        def stage3(g, st):
            logits = []
            for w, (p, pr) in enumerate(st):
                p = p + pr
                if g < w * DIL:
                    pos = row0 + g + _iota((n, LANES), 0)
                    p = jnp.where(pos >= w * DIL, p, -1e9 * math.log2(math.e))
                logits.append(p)
            m = logits[0]
            for w in range(1, WIN):
                m = jnp.maximum(m, logits[w])
            e = [jnp.exp2(l - m) for l in logits]
            den = e[0]
            for w in range(1, WIN):
                den = den + e[w]
            inv = pl.reciprocal(den, approx=True)
            inv = inv * (2.0 - den * inv)
            out = []
            for s in range(NS):
                acc = e[0] * shifted(2 * NS + s, g, 0)
                for w in range(1, WIN):
                    acc = acc + e[w] * shifted(2 * NS + s, g, w)
                out.append(acc * inv)
            return out

        groups = list(range(0, TM, n))
        s1, s2, pend = {}, {}, []
        for t in range(len(groups) + 2):
            if t < len(groups):
                s1[t] = stage1(groups[t])
            if 0 <= t - 1 < len(groups):
                s2[t - 1] = stage2(groups[t - 1], s1.pop(t - 1))
            if 0 <= t - 2 < len(groups):
                pend.append(stage3(groups[t - 2], s2.pop(t - 2)))
                if len(pend) * n >= 16:
                    g0 = groups[t - 2] + n - len(pend) * n
                    for s in range(NS):
                        o = jnp.concatenate([p[s] for p in pend], axis=0)
                        o_s[pl.ds(pl.multiple_of((row0 + g0) // 2, 8), len(pend) * n // 2),
                            s * LANES:(s + 1) * LANES] = pltpu.bitcast(o.astype(BF16), jnp.int32)
                    pend = []
            yield

    def row_dot(x, which):
        p = None
        for s in range(NS):
            w = qkv_s[6 * NS, pl.ds(pl.multiple_of((which + s) * 16, 16), 16), :]
            t = x[:, s * LANES:(s + 1) * LANES] * w
            p = t if p is None else p + t
        return jnp.sum(p, axis=1, keepdims=True)

    def route(first, count, z):
        lane = _iota((8, LANES), 1)
        for i in range(count):
            acc = jnp.full((8, LANES), -jnp.inf, F32)
            for g in range(0, TR, 16):
                rows = pl.ds(pl.multiple_of((first + i) * TR + g, 16), 16)
                x = ax_v[rows, :].astype(F32)
                r = row_dot(x, z)
                acc = jnp.where(lane == g // 8, r[:8], acc)
                acc = jnp.where(lane == g // 8 + 1, r[8:], acc)
                g_s[rows, :] = jnp.broadcast_to(_sigmoid(row_dot(x, z + NS)), (16, LANES))
                if g + 16 == TR:
                    r_s[pl.ds(pl.multiple_of((first + i) * 8, 8), 8), :] = acc
                yield

    wq_cuts = list(range(0, D, UNIT)) + [D]
    wq_parts = list(zip(wq_cuts[:-1], wq_cuts[1:]))
    wq_copy(*wq_parts[0]).start()
    z_s[0] = 0
    for n, ref in enumerate((wr_ref, gw_ref)):
        w = ref[...].astype(F32).reshape(1, D)
        for s in range(NS):
            qkv_s[6 * NS, (n * NS + s) * 16:(n * NS + s + 1) * 16, :] = jnp.broadcast_to(
                w[:, s * LANES:(s + 1) * LANES], (16, LANES))
    tail0, tail = wq_parts[-1][0], D - wq_parts[-1][0]
    dst_col = _iota((D, D), 1)
    perm = jnp.where(_iota((D, D), 0) == (dst_col % H) * DH + dst_col // H, 1.0, 0.0)
    wop_v[...] = pltpu.bitcast(perm.astype(BF16), jnp.int32)
    for part in wq_parts[1:]:
        wq_copy(*part).start()
    with _scope("perm0"):
        wq_copy(*wq_parts[0]).wait()
        ax_copy(0).start()
        permute_unit([(0, 0, UNIT)])
        for part in wq_parts[1:]:
            wq_copy(*part).wait()
        w_copy(1).start()
        permute_mxu(0, tail0, tail)
        permute_unit([(0, UNIT, UNIT)])
    with _scope("w_q0"):
        ax_copy(0).wait()
    with _scope("q0"):
        ax_copy(1).start()
        w_copy(2).start()
        run(project(0, buf_a, 0, NS))
        run(route(0, RPB, 0))
    with _scope("w_q1"):
        w_copy(1).wait()
        ax_copy(1).wait()
    with _scope("q1"):
        ax_copy(2).start()
        ax_copy(3).start()
        run(project(1, buf_b, 0, NS))
        permute_unit([(1, 0, UNIT)])
        permute_unit([(1, UNIT, UNIT)])
        permute_unit([(1, tail0, tail), (1, tail0, tail)])
    with _scope("w_kv0"):
        w_copy(2).wait()
    with _scope("kv0"):
        for i in range(4, NA):
            ax_copy(i).start()
        wg_copy.start()
        wu_copy.start()
        wd_copy.start()
        wo_copy.start()
        fence_copy.start()
        run(project(0, buf_a, NS, 2 * NS))
        permute_unit([(2, 0, UNIT)])
        permute_unit([(2, UNIT, UNIT)])
        permute_unit([(2, tail0, tail), (2, tail0, tail)])
        run(project(0, buf_a, 2 * NS, 3 * NS))
        run(route(RPB, RPB, 0))
        for s in range(NS, 3 * NS):
            qkv_s[s, 0:HALO, :] = jnp.broadcast_to(qkv_s[s, HALO:HALO + 1, :], (HALO, LANES))

    def step_a(i, src, dst, first=False, filler=None):
        for s in range(NS, 3 * NS):
            qkv_s[dst + s, 0:HALO, :] = qkv_s[src + s, TM:TM + HALO, :]
        z = z_s[0]
        jobs = [[attn_block(i - 1, src, z), TM // CH + 2, 0]]
        if filler is None and not first:
            jobs.append([route(2 * RPB + (i - 2) * RPS, RPS, z), RPS * TR // 16, 0])
        lo = NS if first else 0
        n_mm = (3 * NS - lo) * (TM // SP)
        k, lead = 0, (LEAD if filler is None else LEADF)
        for _ in project(i, dst, lo, 3 * NS, filler):
            k += 1
            for job in jobs:
                upto = min(job[1], max(0, round((k - LAG) * job[1] / (n_mm - LAG - lead))))
                for _ in range(upto - job[2]):
                    next(job[0])
                job[2] = upto

    def body_a(j, carry):
        i = 2 * j + 2
        for n in range(2 * RPS // RPB):
            ax_copy(2 + j * (2 * RPS // RPB) + n).wait()
        step_a(i, buf_b, buf_a)
        step_a(i + 1, buf_a, buf_b)
        return carry

    with _scope("step1"):
        step_a(1 + z_s[0], buf_a, buf_b, first=True)
    with _scope("loopA"):
        jax.lax.fori_loop(0, (NA - 4) // 2, body_a, 0)
    wo_copy.wait()
    wg_copy.wait()
    wu_copy.wait()
    wd_copy.wait()

    nr = S // TR * 8
    r = r_s[...].astype(BF16).astype(F32)
    r = jnp.where(r != r, -jnp.inf, r)
    sub = _iota((nr, LANES), 0)
    col = _iota((nr, LANES), 1)
    tok = jnp.where(col < TR // 8, (sub // 8) * TR + col * 8 + sub % 8, S - 1)
    m1 = jnp.max(r)
    i1 = jnp.min(jnp.where(r == m1, tok, S - 1))
    r2 = jnp.where(tok == i1, -jnp.inf, r)
    m2 = jnp.max(r2)
    i2 = jnp.min(jnp.where((r2 == m2) & (tok != i1), tok, S - 1))

    row16 = _iota((16, D), 0)

    def tile_of(i):
        return pl.ds(pl.multiple_of((i // 16) * 16, 16), 16)

    def pick(i):
        tile = ax_v[tile_of(i), :].astype(F32)
        return jnp.sum(jnp.where(row16 == i % 16, tile, 0.0), axis=0, keepdims=True)

    xsel = jnp.where(row16 == 0, pick(i1), jnp.where(row16 == 1, pick(i2), 0.0))
    xsel = xsel.astype(BF16)
    hidden = []

    def ffn_up():
        for _ in range(SKIP):
            yield
        n = NMXU * LANES
        for f0 in range(0, F, n):
            nf = min(n, F - f0)
            if 2 * nf <= n:
                operands = [lambda ks: jnp.concatenate(
                    [wg_v[f0:f0 + nf, ks], wu_v[f0:f0 + nf, ks]], axis=0)]
            else:
                operands = [lambda ks: wg_v[f0:f0 + nf, ks], lambda ks: wu_v[f0:f0 + nf, ks]]
            accs = []
            for operand in operands:
                acc = None
                for k0 in range(0, D, LANES):
                    ks = slice(k0, k0 + LANES)
                    part = _dot_nt(xsel[:, ks], operand(ks))
                    acc = part if acc is None else acc + part
                    yield
                accs.append(acc)
            gg, uu = accs if len(accs) == 2 else (accs[0][:, :nf], accs[0][:, nf:])
            hidden.append((gg * _sigmoid(gg) * uu).astype(BF16))

    filler = ffn_up()
    step_a(NA - 2 + z_s[0], buf_b, buf_a, filler=filler)
    step_a(NA - 1 + z_s[0], buf_a, buf_b, filler=filler)
    run(filler)
    hs_v[...] = jnp.concatenate(hidden, axis=1)
    fence_copy.wait()
    permute_wo()
    y = jnp.dot(hs_v[...], wd_v[...], preferred_element_type=F32)
    attn = attn_block(NA - 1, buf_b, z_s[0])
    for n, (i, m) in enumerate(((i1, m1), (i2, m2))):
        upd = y[n:n + 1, :] * _sigmoid(jnp.full((1, D), m, F32))
        tile = ax_v[tile_of(i), :].astype(F32)
        ax_v[tile_of(i), :] = jnp.where(row16 == i % 16, tile + upd, tile).astype(BF16)

    def out_rows(t, pace):
        row0, row1 = OUT_CUTS[t], OUT_CUTS[t + 1]
        o = pltpu.bitcast(o_s[row0 // 2:row1 // 2, :], BF16)
        a = jnp.dot(o, pltpu.bitcast(wop_v[...], BF16), preferred_element_type=F32)
        for s in range(NS):
            cols = slice(s * LANES, (s + 1) * LANES)
            for r0 in range(0, row1 - row0, SPC):
                rows = slice(row0 + r0, row0 + r0 + SPC)
                g = g_s[rows, :]
                piece = a[r0:r0 + SPC, cols]
                b = ax_v[rows, cols].astype(F32)
                out_v[rows, cols] = (g * piece + (1.0 - g) * b).astype(BF16)
                if pace:
                    qkv_s[6 * NS + 1, r0:r0 + 8, :] = piece[:8]
                yield
        out_copy(t).start()

    n_attn, n_mm = TM // CH + 2, NS * OUT_CUTS[SPREAD] // SPC
    done = k = 0
    for t in range(len(OUT_CUTS) - 1):
        for _ in out_rows(t, t < SPREAD):
            k += 1
            upto = min(n_attn, max(0, round((k - CLAG) * n_attn / (n_mm - CLAG - CLEAD))))
            for _ in range(upto - done):
                next(attn, None)
            done = upto
    with _scope("drain"):
        for t in range(len(OUT_CUTS) - 1):
            out_copy(t).wait()


@jax.jit
def pallas_gated_mix__sliding_local_dilated__moe_arch_mod__prompt_kernel(
    A_x: jax.Array,
    A_wqkv: jax.Array,
    A_wo: jax.Array,
    B_x: jax.Array,
    B_w_r: jax.Array,
    B_w_gate: jax.Array,
    B_w_up: jax.Array,
    B_w_down: jax.Array,
    gate_w: jax.Array,
):
    B, S, D = A_x.shape
    F = B_w_gate.shape[1]
    assert B == 1
    NS = D // LANES
    hbm = pl.BlockSpec(memory_space=pltpu.HBM)
    vmem = pl.BlockSpec(memory_space=pltpu.VMEM)
    out = pl.pallas_call(
        functools.partial(_kernel, S=S, D=D, F=F),
        out_shape=jax.ShapeDtypeStruct((S, D), A_x.dtype),
        in_specs=[hbm, hbm, hbm, vmem, hbm, hbm, hbm, vmem],
        out_specs=hbm,
        scratch_shapes=[
            pltpu.VMEM((S, D), BF16),
            pltpu.VMEM((3, D, D), BF16),
            pltpu.VMEM((D // 2, 3 * D), jnp.int32),
            pltpu.VMEM((D, D), BF16),
            pltpu.VMEM((D // 2, D), jnp.int32),
            pltpu.VMEM((F, D), BF16),
            pltpu.VMEM((F, D), BF16),
            pltpu.VMEM((F, D), BF16),
            pltpu.VMEM((6 * NS + 2, HALO + TM, LANES), F32),
            pltpu.VMEM((S // 2, D), jnp.int32),
            pltpu.VMEM((S, LANES), F32),
            pltpu.SMEM((1,), jnp.int32),
            pltpu.VMEM((S, D), BF16),
            pltpu.VMEM((2, D, LANES), jnp.int32),
            pltpu.VMEM((NS, D, LANES), F32),
            pltpu.VMEM((S // TR * 8, LANES), F32),
            pltpu.VMEM((16, F), BF16),
            pltpu.VMEM((16, D), BF16),
            pltpu.SemaphoreType.DMA((S // TM,)),
            pltpu.SemaphoreType.DMA((6,)),
            pltpu.SemaphoreType.DMA((5,)),
            pltpu.SemaphoreType.DMA((len(OUT_CUTS) - 1,)),
        ],
        compiler_params=pltpu.CompilerParams(vmem_limit_bytes=100 * 2**20, flags=FLAGS),
    )(A_x.reshape(S, D), A_wqkv, A_wo, B_w_r,
      B_w_gate.T, B_w_up.T, B_w_down, gate_w)
    return out.reshape(B, S, D)
```

```python
import contextlib
import functools
import math

import jax
import jax.numpy as jnp
import numpy as np
from jax.experimental import pallas as pl
from jax.experimental.pallas import tpu as pltpu

H = 32
WIN = 8
DIL = 2
HALO = 16
LANES = 128
TM = 256
OUT_CUTS = (0, 256, 512, 768, 1024, 1280, 1536, 1792, 1920, 1984, 2048)
SPREAD = 5
NMXU = 4
SKIP = 4
VCUT = 256
ORDER = 0
RLAG = 12
SPC = 64
CLAG = -1
CLEAD = 1
TR = 128
LEADF = 16
FLAGS = {}
SP = 16
LAG = 0
LEAD = 3
DYNW = 8
CH = 8
F32 = jnp.float32
BF16 = jnp.bfloat16


SCOPES = False


def _scope(name):
    return jax.named_scope(name) if SCOPES else contextlib.nullcontext()


def _sigmoid(x):
    return 0.5 * jnp.tanh(0.5 * x) + 0.5


def _dot_nt(a, b):
    return jax.lax.dot_general(a, b, (((1,), (1,)), ((), ())), preferred_element_type=F32)


def _iota(shape, dim):
    return jax.lax.broadcasted_iota(jnp.int32, shape, dim)


def _kernel(ax_hbm, wqkv_hbm, wo_hbm, wr_v, wg_hbm, wu_hbm, wd_hbm,
            gw_v, out_hbm,
            ax_v, wqkv_v, wp_v, wo_v, wop_v, wg_v, wu_v, wd_v,
            qkv_s, o_s, g_s, z_s, out_v, t_s, two_s, r_s, hs_v, fence_v,
            sem_ax, sem_w, sem_misc, sem_out, *, S, D, F):
    DH = D // H
    NS = D // LANES
    NA = S // TM
    qscale = DH ** -0.5 * math.log2(math.e)
    buf_a, buf_b = 0, 3 * NS
    RPB = TM // TR
    RPS = (NA - 2) * RPB // (NA - 4)
    GRP = LANES // H
    UNIT = 2 * LANES

    def ax_copy(i):
        rows = pl.ds(i * TM, TM)
        return pltpu.make_async_copy(ax_hbm.at[rows], ax_v.at[rows], sem_ax.at[i])

    def w_copy(c, r0, r1):
        rows = pl.ds(r0, r1 - r0)
        return pltpu.make_async_copy(wqkv_hbm.at[rows, pl.ds(c * D, D)], wqkv_v.at[c, rows],
                                     sem_w.at[3 * c + r0 // UNIT])

    wo_copy = pltpu.make_async_copy(wo_hbm, wo_v, sem_misc.at[0])
    wg_copy = pltpu.make_async_copy(wg_hbm, wg_v, sem_misc.at[1])
    wu_copy = pltpu.make_async_copy(wu_hbm, wu_v, sem_misc.at[2])
    wd_copy = pltpu.make_async_copy(wd_hbm, wd_v, sem_misc.at[3])

    fence_copy = pltpu.make_async_copy(ax_hbm.at[pl.ds(0, 16)], fence_v, sem_misc.at[4])

    def out_copy(i):
        rows = pl.ds(OUT_CUTS[i], OUT_CUTS[i + 1] - OUT_CUTS[i])
        return pltpu.make_async_copy(out_v.at[rows], out_hbm.at[rows], sem_out.at[i])

    units = [0]

    def permute_unit(pieces):
        w32 = jnp.concatenate(
            [pltpu.bitcast(wqkv_v[c, r0:r0 + nr, :], jnp.int32) for c, r0, nr in pieces], axis=0)
        tb = units[0] % 2
        units[0] += 1
        t_s[tb] = w32.T
        for s in range(NS):
            parts = [t_s[tb, pl.ds(s * GRP + j, H, stride=DH), :] for j in range(GRP)]
            blk = jnp.concatenate(parts, axis=0).T
            at = 0
            for c, r0, nr in pieces:
                wp_v[r0 // 2:(r0 + nr) // 2,
                     c * D + s * LANES:c * D + (s + 1) * LANES] = blk[at:at + nr // 2]
                at += nr // 2

    def permute_mxu(c, r0, nr):
        blk = jnp.dot(wqkv_v[c, r0:r0 + nr, :], pltpu.bitcast(wop_v[...], BF16),
                      preferred_element_type=F32)
        wp_v[r0 // 2:(r0 + nr) // 2, c * D:(c + 1) * D] = pltpu.bitcast(
            blk.astype(BF16), jnp.int32)

    def permute_wo():
        for s in range(NS):
            cols = slice(s * LANES, (s + 1) * LANES)
            two_s[s] = wo_v[:, cols].astype(F32)
            for d in range(DH):
                rows = two_s[s, pl.ds(d, H, stride=DH), :]
                wop_v[d * H // 2:(d + 1) * H // 2, cols] = pltpu.bitcast(
                    rows.astype(BF16), jnp.int32)

    def project(i, buf, lo, hi, filler=None):
        rows = pl.ds(pl.multiple_of(i * TM, TM), TM)

        def product(k0, k1, c0, c1):
            w = pltpu.bitcast(wp_v[k0 // 2:k1 // 2, c0 * LANES:c1 * LANES], BF16)
            res = jnp.dot(ax_v[rows, k0:k1], w, preferred_element_type=F32)
            if filler is not None:
                next(filler, None)
            return res

        width = hi - lo if filler is None else NMXU
        split = 0 if filler is None else NMXU * LANES
        for c0 in range(lo, hi, width):
            c1 = min(c0 + width, hi)
            rest = product(split, D, c0, c1)
            for s in range(c0, c1):
                res = rest[:, (s - c0) * LANES:(s - c0 + 1) * LANES]
                if split:
                    res = res + product(0, split, s, s + 1)
                if s < NS:
                    res = res * qscale
                for r0 in range(0, TM, SP):
                    qkv_s[buf + s, HALO + r0:HALO + r0 + SP, :] = res[r0:r0 + SP]
                    yield

    def run(gen):
        for _ in gen:
            pass

    def attn_block(i, buf, z):
        row0 = pl.multiple_of(i * TM, TM)
        n = CH

        def shifted(slab, g, w):
            return qkv_s[buf + slab + (z if w >= DYNW else 0),
                         pl.ds(HALO + g - w * DIL, n), :]

        def stage1(g):
            q = [qkv_s[buf + z + s, pl.ds(HALO + g, n), :] for s in range(NS)]
            out = []
            for w in range(WIN):
                p = q[0] * shifted(NS, g, w)
                for s in range(1, NS):
                    p = p + q[s] * shifted(NS + s, g, w)
                out.append((p, pltpu.roll(p, 2 * H, 1)))
            return out

        def stage2(g, st):
            out = []
            for p, pr in st:
                p = p + pr
                out.append((p, pltpu.roll(p, H, 1)))
            return out

        def stage3(g, st):
            logits = []
            for w, (p, pr) in enumerate(st):
                p = p + pr
                if g < w * DIL:
                    pos = row0 + g + _iota((n, LANES), 0)
                    p = jnp.where(pos >= w * DIL, p, -1e9 * math.log2(math.e))
                logits.append(p)
            m = logits[0]
            for w in range(1, WIN):
                m = jnp.maximum(m, logits[w])
            e = [jnp.exp2(l - m) for l in logits]
            den = e[0]
            for w in range(1, WIN):
                den = den + e[w]
            inv = pl.reciprocal(den, approx=True)
            inv = inv * (2.0 - den * inv)
            out = []
            for s in range(NS):
                acc = e[0] * shifted(2 * NS + s, g, 0)
                for w in range(1, WIN):
                    acc = acc + e[w] * shifted(2 * NS + s, g, w)
                out.append(acc * inv)
            return out

        groups = list(range(0, TM, n))
        s1, s2, pend = {}, {}, []
        for t in range(len(groups) + 2):
            if ORDER == 1 and 0 <= t - 1 < len(groups):
                s2[t - 1] = stage2(groups[t - 1], s1.pop(t - 1))
            if t < len(groups):
                s1[t] = stage1(groups[t])
            if ORDER == 0 and 0 <= t - 1 < len(groups):
                s2[t - 1] = stage2(groups[t - 1], s1.pop(t - 1))
            if 0 <= t - 2 < len(groups):
                pend.append(stage3(groups[t - 2], s2.pop(t - 2)))
                if len(pend) * n >= 16:
                    g0 = groups[t - 2] + n - len(pend) * n
                    for s in range(NS):
                        o = jnp.concatenate([p[s] for p in pend], axis=0)
                        o_s[pl.ds(pl.multiple_of((row0 + g0) // 2, 8), len(pend) * n // 2),
                            s * LANES:(s + 1) * LANES] = pltpu.bitcast(o.astype(BF16), jnp.int32)
                    pend = []
            yield

    def row_dot(x, which):
        p = None
        for s in range(NS):
            w = qkv_s[6 * NS, pl.ds(pl.multiple_of((which + s) * 16, 16), 16), :]
            t = x[:, s * LANES:(s + 1) * LANES] * w
            p = t if p is None else p + t
        return jnp.sum(p, axis=1, keepdims=True)

    def route(first, count, z):
        lane = _iota((8, LANES), 1)
        for i in range(count):
            acc = jnp.full((8, LANES), -jnp.inf, F32)
            for g in range(0, TR, 16):
                rows = pl.ds(pl.multiple_of((first + i) * TR + g, 16), 16)
                x = ax_v[rows, :].astype(F32)
                r = row_dot(x, z)
                acc = jnp.where(lane == g // 8, r[:8], acc)
                acc = jnp.where(lane == g // 8 + 1, r[8:], acc)
                g_s[rows, :] = jnp.broadcast_to(_sigmoid(row_dot(x, z + NS)), (16, LANES))
                if g + 16 == TR:
                    r_s[pl.ds(pl.multiple_of((first + i) * 8, 8), 8), :] = acc
                yield

    wq_cuts = list(range(0, D, UNIT)) + [D]
    wq_parts = list(zip(wq_cuts[:-1], wq_cuts[1:]))
    w_copy(0, *wq_parts[0]).start()
    z_s[0] = 0
    tail0, tail = wq_parts[-1][0], D - wq_parts[-1][0]
    dst_col = _iota((D, D), 1)
    perm = jnp.where(_iota((D, D), 0) == (dst_col % H) * DH + dst_col // H, 1.0, 0.0)
    wop_v[...] = pltpu.bitcast(perm.astype(BF16), jnp.int32)
    for part in wq_parts[1:]:
        w_copy(0, *part).start()
    with _scope("perm0"):
        w_copy(0, *wq_parts[0]).wait()
        ax_copy(0).start()
        permute_unit([(0, 0, UNIT)])
        for part in wq_parts[1:]:
            w_copy(0, *part).wait()
        w_copy(1, 0, D).start()
        ax_copy(1).start()
        permute_mxu(0, tail0, tail)
        permute_unit([(0, UNIT, UNIT)])
    with _scope("w_q0"):
        ax_copy(0).wait()
    with _scope("q0"):
        for n, ref in enumerate((wr_v, gw_v)):
            w = ref[...].astype(F32).reshape(1, D)
            for s in range(NS):
                qkv_s[6 * NS, (n * NS + s) * 16:(n * NS + s + 1) * 16, :] = jnp.broadcast_to(
                    w[:, s * LANES:(s + 1) * LANES], (16, LANES))
        w_copy(2, 0, VCUT).start()
        run(project(0, buf_a, 0, NS))
        run(route(0, RPB, 0))
    with _scope("w_q1"):
        w_copy(1, 0, D).wait()
        ax_copy(1).wait()
    with _scope("q1"):
        w_copy(2, VCUT, D).start()
        run(project(1, buf_b, 0, NS))
        permute_unit([(1, 0, UNIT)])
        permute_unit([(1, UNIT, UNIT)])
        permute_unit([(1, tail0, tail), (1, tail0, tail)])
    with _scope("w_kv0"):
        w_copy(2, 0, VCUT).wait()
        w_copy(2, VCUT, D).wait()
    with _scope("kv0"):
        for i in range(2, NA):
            ax_copy(i).start()
        wg_copy.start()
        wu_copy.start()
        wd_copy.start()
        wo_copy.start()
        fence_copy.start()
        run(project(0, buf_a, NS, 2 * NS))
        permute_unit([(2, 0, UNIT)])
        permute_unit([(2, UNIT, UNIT)])
        permute_unit([(2, tail0, tail), (2, tail0, tail)])
        run(project(0, buf_a, 2 * NS, 3 * NS))
        run(route(RPB, RPB, 0))
        for s in range(NS, 3 * NS):
            qkv_s[s, 0:HALO, :] = jnp.broadcast_to(qkv_s[s, HALO:HALO + 1, :], (HALO, LANES))

    def step_a(i, src, dst, first=False, filler=None):
        for s in range(NS, 3 * NS):
            qkv_s[dst + s, 0:HALO, :] = qkv_s[src + s, TM:TM + HALO, :]
        z = z_s[0]
        jobs = [[attn_block(i - 1, src, z), TM // CH + 2, 0]]
        if filler is None and not first:
            jobs.append([route(2 * RPB + (i - 2) * RPS, RPS, z), RPS * TR // 16, 0])
        lo = NS if first else 0
        n_mm = (3 * NS - lo) * (TM // SP)
        k, lead = 0, (LEAD if filler is None else LEADF)
        for _ in project(i, dst, lo, 3 * NS, filler):
            k += 1
            for job in jobs:
                lag = LAG if job is jobs[0] else RLAG
                upto = min(job[1], max(0, round((k - lag) * job[1] / (n_mm - lag - lead))))
                for _ in range(upto - job[2]):
                    next(job[0])
                job[2] = upto

    def body_a(j, carry):
        i = 2 * j + 2
        for n in range(2 * RPS // RPB):
            ax_copy(2 + j * (2 * RPS // RPB) + n).wait()
        step_a(i, buf_b, buf_a)
        step_a(i + 1, buf_a, buf_b)
        return carry

    with _scope("step1"):
        step_a(1 + z_s[0], buf_a, buf_b, first=True)
    with _scope("loopA"):
        jax.lax.fori_loop(0, (NA - 4) // 2, body_a, 0)
    wo_copy.wait()
    wg_copy.wait()
    wu_copy.wait()
    wd_copy.wait()

    nr = S // TR * 8
    r = r_s[...].astype(BF16).astype(F32)
    r = jnp.where(r != r, -jnp.inf, r)
    sub = _iota((nr, LANES), 0)
    col = _iota((nr, LANES), 1)
    tok = jnp.where(col < TR // 8, (sub // 8) * TR + col * 8 + sub % 8, S - 1)
    m1 = jnp.max(r)
    i1 = jnp.min(jnp.where(r == m1, tok, S - 1))
    r2 = jnp.where(tok == i1, -jnp.inf, r)
    m2 = jnp.max(r2)
    i2 = jnp.min(jnp.where((r2 == m2) & (tok != i1), tok, S - 1))

    row16 = _iota((16, D), 0)

    def tile_of(i):
        return pl.ds(pl.multiple_of((i // 16) * 16, 16), 16)

    def pick(i):
        tile = ax_v[tile_of(i), :].astype(F32)
        return jnp.sum(jnp.where(row16 == i % 16, tile, 0.0), axis=0, keepdims=True)

    xsel = jnp.where(row16 == 0, pick(i1), jnp.where(row16 == 1, pick(i2), 0.0))
    xsel = xsel.astype(BF16)
    hidden = []

    def ffn_up():
        for _ in range(SKIP):
            yield
        n = NMXU * LANES
        for f0 in range(0, F, n):
            nf = min(n, F - f0)
            if 2 * nf <= n:
                operands = [lambda ks: jnp.concatenate(
                    [wg_v[f0:f0 + nf, ks], wu_v[f0:f0 + nf, ks]], axis=0)]
            else:
                operands = [lambda ks: wg_v[f0:f0 + nf, ks], lambda ks: wu_v[f0:f0 + nf, ks]]
            accs = []
            for operand in operands:
                acc = None
                for k0 in range(0, D, LANES):
                    ks = slice(k0, k0 + LANES)
                    part = _dot_nt(xsel[:, ks], operand(ks))
                    acc = part if acc is None else acc + part
                    yield
                accs.append(acc)
            gg, uu = accs if len(accs) == 2 else (accs[0][:, :nf], accs[0][:, nf:])
            hidden.append((gg * _sigmoid(gg) * uu).astype(BF16))

    filler = ffn_up()
    step_a(NA - 2 + z_s[0], buf_b, buf_a, filler=filler)
    step_a(NA - 1 + z_s[0], buf_a, buf_b, filler=filler)
    run(filler)
    hs_v[...] = jnp.concatenate(hidden, axis=1)
    fence_copy.wait()
    permute_wo()
    y = jnp.dot(hs_v[...], wd_v[...], preferred_element_type=F32)
    attn = attn_block(NA - 1, buf_b, z_s[0])
    for n, (i, m) in enumerate(((i1, m1), (i2, m2))):
        upd = y[n:n + 1, :] * _sigmoid(jnp.full((1, D), m, F32))
        tile = ax_v[tile_of(i), :].astype(F32)
        ax_v[tile_of(i), :] = jnp.where(row16 == i % 16, tile + upd, tile).astype(BF16)

    def out_rows(t, pace):
        row0, row1 = OUT_CUTS[t], OUT_CUTS[t + 1]
        o = pltpu.bitcast(o_s[row0 // 2:row1 // 2, :], BF16)
        a = jnp.dot(o, pltpu.bitcast(wop_v[...], BF16), preferred_element_type=F32)
        for s in range(NS):
            cols = slice(s * LANES, (s + 1) * LANES)
            for r0 in range(0, row1 - row0, SPC):
                rows = slice(row0 + r0, row0 + r0 + SPC)
                g = g_s[rows, :]
                piece = a[r0:r0 + SPC, cols]
                b = ax_v[rows, cols].astype(F32)
                out_v[rows, cols] = (g * piece + (1.0 - g) * b).astype(BF16)
                if pace:
                    qkv_s[6 * NS + 1, r0:r0 + 8, :] = piece[:8]
                yield
        out_copy(t).start()

    n_attn, n_mm = TM // CH + 2, NS * OUT_CUTS[SPREAD] // SPC
    done = k = 0
    for t in range(len(OUT_CUTS) - 1):
        for _ in out_rows(t, t < SPREAD):
            k += 1
            upto = min(n_attn, max(0, round((k - CLAG) * n_attn / (n_mm - CLAG - CLEAD))))
            for _ in range(upto - done):
                next(attn, None)
            done = upto
    with _scope("drain"):
        for t in range(len(OUT_CUTS) - 1):
            out_copy(t).wait()


@jax.jit
def pallas_gated_mix__sliding_local_dilated__moe_arch_mod__prompt_kernel(
    A_x: jax.Array,
    A_wqkv: jax.Array,
    A_wo: jax.Array,
    B_x: jax.Array,
    B_w_r: jax.Array,
    B_w_gate: jax.Array,
    B_w_up: jax.Array,
    B_w_down: jax.Array,
    gate_w: jax.Array,
):
    B, S, D = A_x.shape
    F = B_w_gate.shape[1]
    assert B == 1
    NS = D // LANES
    hbm = pl.BlockSpec(memory_space=pltpu.HBM)
    vmem = pl.BlockSpec(memory_space=pltpu.VMEM)
    out = pl.pallas_call(
        functools.partial(_kernel, S=S, D=D, F=F),
        out_shape=jax.ShapeDtypeStruct((S, D), A_x.dtype),
        in_specs=[hbm, hbm, hbm, vmem, hbm, hbm, hbm, vmem],
        out_specs=hbm,
        scratch_shapes=[
            pltpu.VMEM((S, D), BF16),
            pltpu.VMEM((3, D, D), BF16),
            pltpu.VMEM((D // 2, 3 * D), jnp.int32),
            pltpu.VMEM((D, D), BF16),
            pltpu.VMEM((D // 2, D), jnp.int32),
            pltpu.VMEM((F, D), BF16),
            pltpu.VMEM((F, D), BF16),
            pltpu.VMEM((F, D), BF16),
            pltpu.VMEM((6 * NS + 2, HALO + TM, LANES), F32),
            pltpu.VMEM((S // 2, D), jnp.int32),
            pltpu.VMEM((S, LANES), F32),
            pltpu.SMEM((1,), jnp.int32),
            pltpu.VMEM((S, D), BF16),
            pltpu.VMEM((2, D, LANES), jnp.int32),
            pltpu.VMEM((NS, D, LANES), F32),
            pltpu.VMEM((S // TR * 8, LANES), F32),
            pltpu.VMEM((16, F), BF16),
            pltpu.VMEM((16, D), BF16),
            pltpu.SemaphoreType.DMA((S // TM,)),
            pltpu.SemaphoreType.DMA((9,)),
            pltpu.SemaphoreType.DMA((5,)),
            pltpu.SemaphoreType.DMA((len(OUT_CUTS) - 1,)),
        ],
        compiler_params=pltpu.CompilerParams(vmem_limit_bytes=100 * 2**20, flags=FLAGS),
    )(A_x.reshape(S, D), A_wqkv, A_wo, B_w_r,
      B_w_gate.T, B_w_up.T, B_w_down, gate_w)
    return out.reshape(B, S, D)
```

```python
import functools
import math

import jax
import jax.numpy as jnp
from jax.experimental import pallas as pl
from jax.experimental.pallas import tpu as pltpu

H = 32
WIN = 8
DIL = 2
HALO = 16
LANES = 128
NMXU = 4
TM = 256
TR = 128
CH = 8
SP = 16
LEAD, LEADF, RLAG = 3, 16, 12
OUT_CUTS = (0, 256, 512, 768, 1024, 1280, 1536, 1792, 1920, 1984, 2016, 2048)
SPREAD = 5
SPC = 32
F32 = jnp.float32
BF16 = jnp.bfloat16


def _sigmoid(x):
    return 0.5 * jnp.tanh(0.5 * x) + 0.5


def _dot_nt(a, b):
    return jax.lax.dot_general(a, b, (((1,), (1,)), ((), ())), preferred_element_type=F32)


def _iota(shape, dim):
    return jax.lax.broadcasted_iota(jnp.int32, shape, dim)


def _kernel(ax_hbm, wqkv_hbm, wo_hbm, wr_v, wg_hbm, wu_hbm, wd_hbm,
            gw_v, out_hbm,
            ax_v, wqkv_v, wp_v, wo_v, wop_v, wg_v, wu_v, wd_v,
            qkv_s, o_s, g_s, z_s, out_v, t_s, two_s, r_s, hs_v, fence_v,
            sem_ax, sem_w, sem_misc, sem_out, *, S, D, F):
    DH = D // H
    NS = D // LANES
    NA = S // TM
    qscale = DH ** -0.5 * math.log2(math.e)
    buf_a, buf_b = 0, 3 * NS
    RPB = TM // TR
    RPS = (NA - 2) * RPB // (NA - 4)
    GRP = LANES // H
    UNIT = 2 * LANES

    def ax_copy(i):
        rows = pl.ds(i * TM, TM)
        return pltpu.make_async_copy(ax_hbm.at[rows], ax_v.at[rows], sem_ax.at[i])

    def w_copy(c, r0, r1):
        rows = pl.ds(r0, r1 - r0)
        return pltpu.make_async_copy(wqkv_hbm.at[rows, pl.ds(c * D, D)], wqkv_v.at[c, rows],
                                     sem_w.at[3 * c + r0 // UNIT])

    wo_copy = pltpu.make_async_copy(wo_hbm, wo_v, sem_misc.at[0])
    wg_copy = pltpu.make_async_copy(wg_hbm, wg_v, sem_misc.at[1])
    wu_copy = pltpu.make_async_copy(wu_hbm, wu_v, sem_misc.at[2])
    wd_copy = pltpu.make_async_copy(wd_hbm, wd_v, sem_misc.at[3])

    fence_copy = pltpu.make_async_copy(ax_hbm.at[pl.ds(0, 16)], fence_v, sem_misc.at[4])

    def out_copy(i):
        rows = pl.ds(OUT_CUTS[i], OUT_CUTS[i + 1] - OUT_CUTS[i])
        return pltpu.make_async_copy(out_v.at[rows], out_hbm.at[rows], sem_out.at[i])

    units = [0]

    def permute_unit(pieces):
        w32 = jnp.concatenate(
            [pltpu.bitcast(wqkv_v[c, r0:r0 + nr, :], jnp.int32) for c, r0, nr in pieces], axis=0)
        tb = units[0] % 2
        units[0] += 1
        t_s[tb] = w32.T
        for s in range(NS):
            parts = [t_s[tb, pl.ds(s * GRP + j, H, stride=DH), :] for j in range(GRP)]
            blk = jnp.concatenate(parts, axis=0).T
            at = 0
            for c, r0, nr in pieces:
                wp_v[r0 // 2:(r0 + nr) // 2,
                     c * D + s * LANES:c * D + (s + 1) * LANES] = blk[at:at + nr // 2]
                at += nr // 2

    def permute_mxu(c, r0, nr):
        blk = jnp.dot(wqkv_v[c, r0:r0 + nr, :], pltpu.bitcast(wop_v[...], BF16),
                      preferred_element_type=F32)
        wp_v[r0 // 2:(r0 + nr) // 2, c * D:(c + 1) * D] = pltpu.bitcast(
            blk.astype(BF16), jnp.int32)

    def permute_wo():
        for s in range(NS):
            cols = slice(s * LANES, (s + 1) * LANES)
            two_s[s] = wo_v[:, cols].astype(F32)
            for d in range(DH):
                rows = two_s[s, pl.ds(d, H, stride=DH), :]
                wop_v[d * H // 2:(d + 1) * H // 2, cols] = pltpu.bitcast(
                    rows.astype(BF16), jnp.int32)

    def project(i, buf, lo, hi, filler=None):
        rows = pl.ds(pl.multiple_of(i * TM, TM), TM)

        def product(k0, k1, c0, c1):
            w = pltpu.bitcast(wp_v[k0 // 2:k1 // 2, c0 * LANES:c1 * LANES], BF16)
            res = jnp.dot(ax_v[rows, k0:k1], w, preferred_element_type=F32)
            if filler is not None:
                next(filler, None)
            return res

        width = hi - lo if filler is None else NMXU
        split = 0 if filler is None else NMXU * LANES
        for c0 in range(lo, hi, width):
            c1 = min(c0 + width, hi)
            rest = product(split, D, c0, c1)
            for s in range(c0, c1):
                res = rest[:, (s - c0) * LANES:(s - c0 + 1) * LANES]
                if split:
                    res = res + product(0, split, s, s + 1)
                if s < NS:
                    res = res * qscale
                for r0 in range(0, TM, SP):
                    qkv_s[buf + s, HALO + r0:HALO + r0 + SP, :] = res[r0:r0 + SP]
                    yield

    def run(gen):
        for _ in gen:
            pass

    def attn_block(i, buf, z):
        row0 = pl.multiple_of(i * TM, TM)
        n = CH

        def shifted(slab, g, w):
            return qkv_s[buf + slab, pl.ds(HALO + g - w * DIL, n), :]

        def stage1(g):
            q = [qkv_s[buf + z + s, pl.ds(HALO + g, n), :] for s in range(NS)]
            out = []
            for w in range(WIN):
                p = q[0] * shifted(NS, g, w)
                for s in range(1, NS):
                    p = p + q[s] * shifted(NS + s, g, w)
                out.append((p, pltpu.roll(p, 2 * H, 1)))
            return out

        def stage2(g, st):
            out = []
            for p, pr in st:
                p = p + pr
                out.append((p, pltpu.roll(p, H, 1)))
            return out

        def stage3(g, st):
            logits = []
            for w, (p, pr) in enumerate(st):
                p = p + pr
                if g < w * DIL:
                    pos = row0 + g + _iota((n, LANES), 0)
                    p = jnp.where(pos >= w * DIL, p, -1e9 * math.log2(math.e))
                logits.append(p)
            m = logits[0]
            for w in range(1, WIN):
                m = jnp.maximum(m, logits[w])
            e = [jnp.exp2(l - m) for l in logits]
            den = e[0]
            for w in range(1, WIN):
                den = den + e[w]
            inv = pl.reciprocal(den, approx=True)
            inv = inv * (2.0 - den * inv)
            out = []
            for s in range(NS):
                acc = e[0] * shifted(2 * NS + s, g, 0)
                for w in range(1, WIN):
                    acc = acc + e[w] * shifted(2 * NS + s, g, w)
                out.append(acc * inv)
            return out

        groups = list(range(0, TM, n))
        s1, s2, pend = {}, {}, []
        for t in range(len(groups) + 2):
            if t < len(groups):
                s1[t] = stage1(groups[t])
            if 0 <= t - 1 < len(groups):
                s2[t - 1] = stage2(groups[t - 1], s1.pop(t - 1))
            if 0 <= t - 2 < len(groups):
                pend.append(stage3(groups[t - 2], s2.pop(t - 2)))
                if len(pend) * n >= 16:
                    g0 = groups[t - 2] + n - len(pend) * n
                    for s in range(NS):
                        o = jnp.concatenate([p[s] for p in pend], axis=0)
                        o_s[pl.ds(pl.multiple_of((row0 + g0) // 2, 8), len(pend) * n // 2),
                            s * LANES:(s + 1) * LANES] = pltpu.bitcast(o.astype(BF16), jnp.int32)
                    pend = []
            yield

    def row_dot(x, which):
        p = None
        for s in range(NS):
            w = qkv_s[6 * NS, pl.ds(pl.multiple_of((which + s) * 16, 16), 16), :]
            t = x[:, s * LANES:(s + 1) * LANES] * w
            p = t if p is None else p + t
        return jnp.sum(p, axis=1, keepdims=True)

    def route(first, count, z):
        lane = _iota((8, LANES), 1)
        for i in range(count):
            acc = jnp.full((8, LANES), -jnp.inf, F32)
            for g in range(0, TR, 16):
                rows = pl.ds(pl.multiple_of((first + i) * TR + g, 16), 16)
                x = ax_v[rows, :].astype(F32)
                r = row_dot(x, z)
                acc = jnp.where(lane == g // 8, r[:8], acc)
                acc = jnp.where(lane == g // 8 + 1, r[8:], acc)
                g_s[rows, :] = jnp.broadcast_to(_sigmoid(row_dot(x, z + NS)), (16, LANES))
                if g + 16 == TR:
                    r_s[pl.ds(pl.multiple_of((first + i) * 8, 8), 8), :] = acc
                yield

    wq_cuts = list(range(0, D, UNIT)) + [D]
    wq_parts = list(zip(wq_cuts[:-1], wq_cuts[1:]))
    w_copy(0, *wq_parts[0]).start()
    z_s[0] = 0
    tail0, tail = wq_parts[-1][0], D - wq_parts[-1][0]
    dst_col = _iota((D, D), 1)
    perm = jnp.where(_iota((D, D), 0) == (dst_col % H) * DH + dst_col // H, 1.0, 0.0)
    wop_v[...] = pltpu.bitcast(perm.astype(BF16), jnp.int32)
    for part in wq_parts[1:]:
        w_copy(0, *part).start()
    w_copy(0, *wq_parts[0]).wait()
    ax_copy(0).start()
    permute_unit([(0, 0, UNIT)])
    for part in wq_parts[1:]:
        w_copy(0, *part).wait()
    w_copy(1, 0, D).start()
    ax_copy(1).start()
    permute_mxu(0, tail0, tail)
    permute_unit([(0, UNIT, UNIT)])
    ax_copy(0).wait()
    for n, ref in enumerate((wr_v, gw_v)):
        w = ref[...].astype(F32).reshape(1, D)
        for s in range(NS):
            qkv_s[6 * NS, (n * NS + s) * 16:(n * NS + s + 1) * 16, :] = jnp.broadcast_to(
                w[:, s * LANES:(s + 1) * LANES], (16, LANES))
    w_copy(2, 0, UNIT).start()
    run(project(0, buf_a, 0, NS))
    run(route(0, RPB, 0))
    w_copy(1, 0, D).wait()
    ax_copy(1).wait()
    w_copy(2, UNIT, D).start()
    run(project(1, buf_b, 0, NS))
    permute_unit([(1, 0, UNIT)])
    permute_unit([(1, UNIT, UNIT)])
    permute_unit([(1, tail0, tail), (1, tail0, tail)])
    w_copy(2, 0, UNIT).wait()
    w_copy(2, UNIT, D).wait()
    for i in range(2, NA):
        ax_copy(i).start()
    wg_copy.start()
    wu_copy.start()
    wd_copy.start()
    wo_copy.start()
    fence_copy.start()
    run(project(0, buf_a, NS, 2 * NS))
    permute_unit([(2, 0, UNIT)])
    permute_unit([(2, UNIT, UNIT)])
    permute_unit([(2, tail0, tail), (2, tail0, tail)])
    run(project(0, buf_a, 2 * NS, 3 * NS))
    run(route(RPB, RPB, 0))
    for s in range(NS, 3 * NS):
        qkv_s[s, 0:HALO, :] = jnp.broadcast_to(qkv_s[s, HALO:HALO + 1, :], (HALO, LANES))

    def step_a(i, src, dst, first=False, filler=None):
        for s in range(NS, 3 * NS):
            qkv_s[dst + s, 0:HALO, :] = qkv_s[src + s, TM:TM + HALO, :]
        z = z_s[0]
        jobs = [[attn_block(i - 1, src, z), TM // CH + 2, 0]]
        if filler is None and not first:
            jobs.append([route(2 * RPB + (i - 2) * RPS, RPS, z), RPS * TR // 16, 0])
        lo = NS if first else 0
        n_mm = (3 * NS - lo) * (TM // SP)
        k, lead = 0, (LEAD if filler is None else LEADF)
        for _ in project(i, dst, lo, 3 * NS, filler):
            k += 1
            for job in jobs:
                lag = 0 if job is jobs[0] else RLAG
                upto = min(job[1], max(0, round((k - lag) * job[1] / (n_mm - lag - lead))))
                for _ in range(upto - job[2]):
                    next(job[0])
                job[2] = upto

    def body_a(j, carry):
        i = 2 * j + 2
        for n in range(2 * RPS // RPB):
            ax_copy(2 + j * (2 * RPS // RPB) + n).wait()
        step_a(i, buf_b, buf_a)
        step_a(i + 1, buf_a, buf_b)
        return carry

    step_a(1 + z_s[0], buf_a, buf_b, first=True)
    jax.lax.fori_loop(0, (NA - 4) // 2, body_a, 0)
    wo_copy.wait()
    wg_copy.wait()
    wu_copy.wait()
    wd_copy.wait()

    nr = S // TR * 8
    r = r_s[...].astype(BF16).astype(F32)
    r = jnp.where(r != r, -jnp.inf, r)
    sub = _iota((nr, LANES), 0)
    col = _iota((nr, LANES), 1)
    tok = jnp.where(col < TR // 8, (sub // 8) * TR + col * 8 + sub % 8, S - 1)
    m1 = jnp.max(r)
    i1 = jnp.min(jnp.where(r == m1, tok, S - 1))
    r2 = jnp.where(tok == i1, -jnp.inf, r)
    m2 = jnp.max(r2)
    i2 = jnp.min(jnp.where((r2 == m2) & (tok != i1), tok, S - 1))

    row16 = _iota((16, D), 0)

    def tile_of(i):
        return pl.ds(pl.multiple_of((i // 16) * 16, 16), 16)

    def pick(i):
        tile = ax_v[tile_of(i), :].astype(F32)
        return jnp.sum(jnp.where(row16 == i % 16, tile, 0.0), axis=0, keepdims=True)

    xsel = jnp.where(row16 == 0, pick(i1), jnp.where(row16 == 1, pick(i2), 0.0))
    xsel = xsel.astype(BF16)
    hidden = []

    def ffn_up():
        for _ in range(NMXU):
            yield
        n = NMXU * LANES
        for f0 in range(0, F, n):
            nf = min(n, F - f0)
            if 2 * nf <= n:
                operands = [lambda ks: jnp.concatenate(
                    [wg_v[f0:f0 + nf, ks], wu_v[f0:f0 + nf, ks]], axis=0)]
            else:
                operands = [lambda ks: wg_v[f0:f0 + nf, ks], lambda ks: wu_v[f0:f0 + nf, ks]]
            accs = []
            for operand in operands:
                acc = None
                for k0 in range(0, D, LANES):
                    ks = slice(k0, k0 + LANES)
                    part = _dot_nt(xsel[:, ks], operand(ks))
                    acc = part if acc is None else acc + part
                    yield
                accs.append(acc)
            gg, uu = accs if len(accs) == 2 else (accs[0][:, :nf], accs[0][:, nf:])
            hidden.append((gg * _sigmoid(gg) * uu).astype(BF16))

    filler = ffn_up()
    step_a(NA - 2 + z_s[0], buf_b, buf_a, filler=filler)
    step_a(NA - 1 + z_s[0], buf_a, buf_b, filler=filler)
    run(filler)
    hs_v[...] = jnp.concatenate(hidden, axis=1)
    fence_copy.wait()
    permute_wo()
    y = jnp.dot(hs_v[...], wd_v[...], preferred_element_type=F32)
    attn = attn_block(NA - 1, buf_b, z_s[0])
    for n, (i, m) in enumerate(((i1, m1), (i2, m2))):
        upd = y[n:n + 1, :] * _sigmoid(jnp.full((1, D), m, F32))
        tile = ax_v[tile_of(i), :].astype(F32)
        ax_v[tile_of(i), :] = jnp.where(row16 == i % 16, tile + upd, tile).astype(BF16)

    def out_rows(t, pace):
        row0, row1 = OUT_CUTS[t], OUT_CUTS[t + 1]
        o = pltpu.bitcast(o_s[row0 // 2:row1 // 2, :], BF16)
        a = jnp.dot(o, pltpu.bitcast(wop_v[...], BF16), preferred_element_type=F32)
        for s in range(NS):
            cols = slice(s * LANES, (s + 1) * LANES)
            for r0 in range(0, row1 - row0, SPC):
                rows = slice(row0 + r0, row0 + r0 + SPC)
                g = g_s[rows, :]
                piece = a[r0:r0 + SPC, cols]
                b = ax_v[rows, cols].astype(F32)
                out_v[rows, cols] = (g * piece + (1.0 - g) * b).astype(BF16)
                if pace:
                    qkv_s[6 * NS + 1, r0:r0 + 8, :] = piece[:8]
                yield
        out_copy(t).start()

    n_attn, n_mm = TM // CH + 2, NS * OUT_CUTS[SPREAD] // SPC
    done = k = 0
    for t in range(len(OUT_CUTS) - 1):
        for _ in out_rows(t, t < SPREAD):
            k += 1
            upto = min(n_attn, max(0, round((k + 1) * n_attn / n_mm)))
            for _ in range(upto - done):
                next(attn, None)
            done = upto
    for t in range(len(OUT_CUTS) - 1):
        out_copy(t).wait()


@jax.jit
def pallas_gated_mix__sliding_local_dilated__moe_arch_mod__prompt_kernel(
    A_x: jax.Array,
    A_wqkv: jax.Array,
    A_wo: jax.Array,
    B_x: jax.Array,
    B_w_r: jax.Array,
    B_w_gate: jax.Array,
    B_w_up: jax.Array,
    B_w_down: jax.Array,
    gate_w: jax.Array,
):
    B, S, D = A_x.shape
    F = B_w_gate.shape[1]
    assert B == 1
    NS = D // LANES
    hbm = pl.BlockSpec(memory_space=pltpu.HBM)
    vmem = pl.BlockSpec(memory_space=pltpu.VMEM)
    out = pl.pallas_call(
        functools.partial(_kernel, S=S, D=D, F=F),
        out_shape=jax.ShapeDtypeStruct((S, D), A_x.dtype),
        in_specs=[hbm, hbm, hbm, vmem, hbm, hbm, hbm, vmem],
        out_specs=hbm,
        scratch_shapes=[
            pltpu.VMEM((S, D), BF16),
            pltpu.VMEM((3, D, D), BF16),
            pltpu.VMEM((D // 2, 3 * D), jnp.int32),
            pltpu.VMEM((D, D), BF16),
            pltpu.VMEM((D // 2, D), jnp.int32),
            pltpu.VMEM((F, D), BF16),
            pltpu.VMEM((F, D), BF16),
            pltpu.VMEM((F, D), BF16),
            pltpu.VMEM((6 * NS + 2, HALO + TM, LANES), F32),
            pltpu.VMEM((S // 2, D), jnp.int32),
            pltpu.VMEM((S, LANES), F32),
            pltpu.SMEM((1,), jnp.int32),
            pltpu.VMEM((S, D), BF16),
            pltpu.VMEM((2, D, LANES), jnp.int32),
            pltpu.VMEM((NS, D, LANES), F32),
            pltpu.VMEM((S // TR * 8, LANES), F32),
            pltpu.VMEM((16, F), BF16),
            pltpu.VMEM((16, D), BF16),
            pltpu.SemaphoreType.DMA((S // TM,)),
            pltpu.SemaphoreType.DMA((9,)),
            pltpu.SemaphoreType.DMA((5,)),
            pltpu.SemaphoreType.DMA((len(OUT_CUTS) - 1,)),
        ],
        compiler_params=pltpu.CompilerParams(vmem_limit_bytes=100 * 2**20),
    )(A_x.reshape(S, D), A_wqkv, A_wo, B_w_r,
      B_w_gate.T, B_w_up.T, B_w_down, gate_w)
    return out.reshape(B, S, D)
```
